```python
import jax
import jax.numpy as jnp

def _softmax(x, axis=-1):
    return jax.nn.softmax(x, axis=axis)

def _gelu(x):
    return jax.nn.gelu(x, approximate=True)

def _silu(x):
    return jax.nn.silu(x)

def _sigmoid(x):
    return jax.nn.sigmoid(x)

def _layernorm(x, axis=-1, eps=1e-05):
    m = jnp.mean(x, axis=axis, keepdims=True)
    v = jnp.var(x, axis=axis, keepdims=True)
    return (x - m) / jnp.sqrt(v + eps)

def _scatter_add(tgt, idx, src, axis=0):
    return tgt.at[idx].add(src)

def _segment_sum(src, seg, n):
    return jax.ops.segment_sum(src, seg, n)

class _Rng:

    def __init__(self, key):
        self._k = key

    def _next(self):
        self._k, sub = jax.random.split(self._k)
        return sub

    def normal(self, shape):
        return jax.random.normal(self._next(), shape, dtype=jnp.bfloat16)

    def randint(self, lo, hi, shape):
        return jax.random.randint(self._next(), shape, lo, hi, dtype=jnp.int32)

    def uniform(self, shape, lo=0.0, hi=1.0):
        return jax.random.uniform(self._next(), shape, jnp.bfloat16, lo, hi)

    def permutation(self, n):
        return jax.random.permutation(self._next(), n)
kernel_name = 'interleave_layers__memory_aug_recurrent_mem_tr__sliding_local_dilated__prompt'

def setup_inputs():
    _rng = _Rng(jax.random.key(int.from_bytes(__import__("os").urandom(4), "little")))
    _w = lambda a: (lambda t: t.astype(jnp.bfloat16) if jnp.issubdtype(t.dtype, jnp.floating) else t)(jnp.asarray(a))

    def _A_setup():
        B, S, Dm = (1, 2048, 640)
        H, Dh = (32, 192)
        M, seg = (8, 32)
        seg = min(seg, S)
        S = S // seg * seg
        return {'x': _w((lambda *s: _rng.normal(s) * 0.05)(B, S, Dm)), 'mem0': _w((lambda *s: _rng.normal(s) * 0.05)(B, M, Dm)), 'Wq': _w((lambda *s: _rng.normal(s) * 0.05)(Dm, H, Dh) * Dm ** (-0.5)), 'Wk': _w((lambda *s: _rng.normal(s) * 0.05)(Dm, H, Dh) * Dm ** (-0.5)), 'Wv': _w((lambda *s: _rng.normal(s) * 0.05)(Dm, H, Dh) * Dm ** (-0.5)), 'Wo': _w((lambda *s: _rng.normal(s) * 0.05)(H, Dh, Dm) * (H * Dh) ** (-0.5)), 'seg_len': seg}
    _A_in = _A_setup()

    def _B_setup():
        B, S, D = (1, 2048, 640)
        return {'x': _w((lambda *s: _rng.normal(s) * 0.05)(B, S, D)), 'wqkv': _w((lambda *s: _rng.normal(s) * 0.05)(D, 3 * D)), 'wo': _w((lambda *s: _rng.normal(s) * 0.05)(D, D))}
    _B_in = _B_setup()
    return {'A_x': _A_in['x'], 'A_mem0': _A_in['mem0'], 'A_Wq': _A_in['Wq'], 'A_Wk': _A_in['Wk'], 'A_Wv': _A_in['Wv'], 'A_Wo': _A_in['Wo'], 'A_seg_len': _A_in['seg_len'], 'B_x': _B_in['x'], 'B_wqkv': _B_in['wqkv'], 'B_wo': _B_in['wo']}

def reference(A_x, A_mem0, A_Wq, A_Wk, A_Wv, A_Wo, A_seg_len, B_x, B_wqkv, B_wo):

    def _A_ref(x, mem0, Wq, Wk, Wv, Wo, seg_len):
        B, S, Dm = x.shape
        H, Dh = (Wq.shape[1], Wq.shape[2])
        M = mem0.shape[1]
        scale = Dh ** (-0.5)
        n_seg = S // seg_len
        L = M + seg_len
        idx = jnp.arange(L)
        mask = (idx[:, None] < M) | (idx[:, None] >= idx[None, :])
        mem = mem0
        outs = []
        for s in range(n_seg):
            xs = x[:, s * seg_len:(s + 1) * seg_len, :].copy()
            h = jnp.concatenate([mem, xs], axis=1)
            q = jnp.einsum('btd,dhe->bhte', h, Wq)
            k = jnp.einsum('btd,dhe->bhte', h, Wk)
            v = jnp.einsum('btd,dhe->bhte', h, Wv)
            scores = jnp.einsum('bhqe,bhke->bhqk', q, k) * scale
            scores = jnp.where(mask[None, None], scores, -1000000000.0)
            p = _softmax(scores, axis=-1)
            o = jnp.einsum('bhqk,bhke->bhqe', p, v)
            o = jnp.einsum('bhte,hed->btd', o, Wo)
            mem = o[:, :M, :].copy()
            outs.append(o[:, M:, :])
        return jnp.concatenate(outs, axis=1)

    def _B_ref(x, wqkv, wo):
        B, S, D = x.shape
        H = 32
        Dh = D // H
        W, dil = (8, 2)
        qkv = (lambda x, *d: x.transpose(*d))((x @ wqkv).reshape(B, S, 3, H, Dh), 2, 0, 3, 1, 4)
        q, k, v = (qkv[0], qkv[1], qkv[2])
        scale = Dh ** (-0.5)
        pos = jnp.arange(S)
        off = jnp.arange(W) * dil
        idx = pos[:, None] - off[None, :]
        mask = idx >= 0
        idx_c = jnp.where(mask, idx, 0).reshape(-1)
        kg = k[:, :, idx_c, :].reshape(B, H, S, W, Dh)
        vg = v[:, :, idx_c, :].reshape(B, H, S, W, Dh)
        logits = jnp.einsum('bhsd,bhswd->bhsw', q, kg) * scale
        logits = jnp.where(mask[None, None, :, :], logits, -1000000000.0)
        attn = _softmax(logits, axis=-1)
        o = jnp.einsum('bhsw,bhswd->bhsd', attn, vg)
        return (lambda x, *d: x.transpose(*d))(o, 0, 2, 1, 3).reshape(B, S, D) @ wo
    x = A_x
    x = x + _A_ref(_layernorm(x, axis=-1), A_mem0, A_Wq, A_Wk, A_Wv, A_Wo, A_seg_len)
    x = x + _B_ref(_layernorm(x, axis=-1), B_wqkv, B_wo)
    x = x + _A_ref(_layernorm(x, axis=-1), A_mem0, A_Wq, A_Wk, A_Wv, A_Wo, A_seg_len)
    x = x + _B_ref(_layernorm(x, axis=-1), B_wqkv, B_wo)
    return x
```

```python
import functools
import jax
import jax.numpy as jnp
from jax import lax
from jax.experimental import pallas as pl
from jax.experimental.pallas import tpu as pltpu

F32 = jnp.float32
BF16 = jnp.bfloat16
NT_DIMS = (((1,), (1,)), ((), ()))
NEG = -1e9
EPS = 1e-5


def _ln(xf):
    m = jnp.mean(xf, axis=-1, keepdims=True)
    d = xf - m
    v = jnp.mean(d * d, axis=-1, keepdims=True)
    return d * lax.rsqrt(v + EPS)


def _dot(a, b):
    return jnp.dot(a, b, preferred_element_type=F32)


def _dot_nt(a, b):
    return lax.dot_general(a, b, NT_DIMS, preferred_element_type=F32)


def _kernel(x_ref, mem0_ref, wq_ref, wk_ref, wv_ref, wo_ref, bw_ref, bo_ref, out_ref,
            r_ref, h_ref, q_ref, k_ref, v_ref, o_ref, bwp_ref, bop_ref, kb_ref, vb_ref,
            *, S, D, H, DH, M, SEG, BH, BW, BDIL):
    NS = S // SEG
    NP = H // 2
    PW = 2 * DH
    R2 = 2 * M + 2 * SEG
    PAD = 3
    BDH = D // BH
    HALO = 16

    rr = lax.broadcasted_iota(jnp.int32, (D, D), 0)
    cc = lax.broadcasted_iota(jnp.int32, (D, D), 1)
    src_of_c = (cc % BH) * BDH + cc // BH
    perm = jnp.where(rr == src_of_c, 1.0, 0.0).astype(BF16)
    src_of_r = (rr % BH) * BDH + rr // BH
    permT = jnp.where(cc == src_of_r, 1.0, 0.0).astype(BF16)
    for i in range(3):
        bwp_ref[:, i * D:(i + 1) * D] = _dot(bw_ref[:, i * D:(i + 1) * D], perm).astype(BF16)
    bop_ref[...] = _dot(permT, bo_ref[...]).astype(BF16)

    r_ref[0:PAD * SEG, :] = jnp.zeros((PAD * SEG, D), BF16)
    r_ref[(PAD + NS) * SEG:(2 * PAD + NS) * SEG, :] = jnp.zeros((PAD * SEG, D), BF16)
    r_ref[PAD * SEG:(PAD + NS) * SEG, :] = x_ref[...]
    kb_ref[...] = jnp.zeros(kb_ref.shape, F32)
    vb_ref[...] = jnp.zeros(vb_ref.shape, F32)

    mem0 = mem0_ref[...].astype(F32)
    mem00 = jnp.concatenate([mem0, mem0], axis=0)
    h_ref[0, 0:2 * M, :] = mem00.astype(BF16)
    h_ref[0, 2 * M:2 * M + SEG, :] = _ln(x_ref[0:SEG, :].astype(F32)).astype(BF16)
    h_ref[0, 2 * M + SEG:R2, :] = jnp.zeros((SEG, D), BF16)

    a_scale = DH ** -0.5
    b_scale = BDH ** -0.5

    def seg(i):
        return pl.ds(pl.multiple_of((i + PAD) * SEG, SEG), SEG)

    def step(t, _):
        slot = lax.rem(t, 2)
        nslot = 1 - slot
        hrows = h_ref[slot]

        ri = lax.broadcasted_iota(jnp.int32, (R2, R2), 0)
        ci = lax.broadcasted_iota(jnp.int32, (R2, R2), 1)
        def layer(i):
            return jnp.where(i < M, 0, jnp.where(i < 2 * M, 1, jnp.where(i < 2 * M + SEG, 0, 1)))
        amask = (layer(ri) == layer(ci)) & ((ri < 2 * M) | (ci < 2 * M) | (ri >= ci))
        lo = lax.broadcasted_iota(jnp.int32, (R2, 128), 1) < 64

        q_ref[...] = _dot_nt(hrows, wq_ref[...]).astype(BF16)
        k_ref[...] = _dot_nt(hrows, wk_ref[...]).astype(BF16)
        v_ref[...] = _dot_nt(hrows, wv_ref[...]).astype(BF16)

        for p in range(NP):
            c0 = p * PW
            qA = q_ref[:, c0:c0 + 128]
            qB = q_ref[:, c0 + 128:c0 + 256]
            qC = q_ref[:, c0 + 256:c0 + 384]
            zero = jnp.zeros_like(qB)
            q0 = jnp.concatenate([qA, jnp.where(lo, qB, zero)], axis=1)
            q1 = jnp.concatenate([jnp.where(lo, zero, qB), qC], axis=1)
            s0 = _dot_nt(q0, k_ref[:, c0:c0 + 256])
            s1 = _dot_nt(q1, k_ref[:, c0 + 128:c0 + 384])
            ps = []
            for s in (s0, s1):
                s = jnp.where(amask, s * a_scale, NEG)
                mx = jnp.max(s, axis=-1, keepdims=True)
                e = jnp.exp(s - mx)
                sm = jnp.sum(e, axis=-1, keepdims=True)
                ps.append((e / sm).astype(BF16))
            o0 = _dot(ps[0], v_ref[:, c0:c0 + 256])
            o1 = _dot(ps[1], v_ref[:, c0 + 128:c0 + 384])
            oB = jnp.where(lo, o0[:, 128:256], o1[:, 0:128])
            o_ref[:, c0:c0 + 128] = o0[:, 0:128].astype(BF16)
            o_ref[:, c0 + 128:c0 + 256] = oB.astype(BF16)
            o_ref[:, c0 + 256:c0 + 384] = o1[:, 128:256].astype(BF16)

        aout = _dot(o_ref[...], wo_ref[...])
        r_ref[seg(t), :] = (r_ref[seg(t), :].astype(F32) + aout[2 * M:2 * M + SEG]).astype(BF16)
        r_ref[seg(t - 2), :] = (r_ref[seg(t - 2), :].astype(F32) + aout[2 * M + SEG:R2]).astype(BF16)
        mrow = lax.broadcasted_iota(jnp.int32, (2 * M, D), 0)
        keep = (mrow < M) | (t >= 2)
        h_ref[nslot, 0:2 * M, :] = jnp.where(keep, aout[0:2 * M], mem00).astype(BF16)
        h_ref[nslot, 2 * M:2 * M + SEG, :] = _ln(r_ref[seg(t + 1), :].astype(F32)).astype(BF16)

        xb0 = r_ref[seg(t - 1), :].astype(F32)
        xb1 = r_ref[seg(t - 3), :].astype(F32)
        xb = jnp.concatenate([xb0, xb1], axis=0)
        hb = _ln(xb).astype(BF16)
        qkv = _dot(hb, bwp_ref[...])
        obs = []
        for l, sidx in enumerate((t - 1, t - 3)):
            rows = slice(l * SEG, (l + 1) * SEG)
            qb = qkv[rows, 0:D] * b_scale
            kb_ref[l, 0:HALO, :] = kb_ref[l, SEG:SEG + HALO, :]
            vb_ref[l, 0:HALO, :] = vb_ref[l, SEG:SEG + HALO, :]
            kb_ref[l, HALO:HALO + SEG, :] = qkv[rows, D:2 * D]
            vb_ref[l, HALO:HALO + SEG, :] = qkv[rows, 2 * D:3 * D]
            pos = lax.broadcasted_iota(jnp.int32, (SEG, 128), 0) + sidx * SEG
            logits = []
            for w in range(BW):
                ks = kb_ref[l, HALO - BDIL * w:HALO - BDIL * w + SEG, :]
                pr = qb * ks
                a = pr[:, 0:128]
                for c in range(1, D // 128):
                    a = a + pr[:, c * 128:(c + 1) * 128]
                a = a + pltpu.roll(a, 64, 1)
                a = a + pltpu.roll(a, 32, 1)
                logits.append(jnp.where(pos >= BDIL * w, a, NEG))
            mx = logits[0]
            for w in range(1, BW):
                mx = jnp.maximum(mx, logits[w])
            es = [jnp.exp(a - mx) for a in logits]
            sm = es[0]
            for w in range(1, BW):
                sm = sm + es[w]
            inv = 1.0 / sm
            ob = None
            for w in range(BW):
                vs = vb_ref[l, HALO - BDIL * w:HALO - BDIL * w + SEG, :]
                aw = es[w] * inv
                aw5 = jnp.concatenate([aw] * (D // 128), axis=1)
                ob = aw5 * vs if ob is None else ob + aw5 * vs
            obs.append(ob)
        ob = jnp.concatenate(obs, axis=0).astype(BF16)
        bout = _dot(ob, bop_ref[...])
        xn = xb + bout
        r_ref[seg(t - 1), :] = xn[0:SEG].astype(BF16)
        r_ref[seg(t - 3), :] = xn[SEG:2 * SEG].astype(BF16)
        h_ref[nslot, 2 * M + SEG:R2, :] = _ln(r_ref[seg(t - 1), :].astype(F32)).astype(BF16)
        return 0

    lax.fori_loop(0, NS + 3, step, 0)
    out_ref[...] = r_ref[PAD * SEG:(PAD + NS) * SEG, :]


@functools.partial(jax.jit, static_argnames=("A_seg_len",))
def pallas_interleave_layers__memory_aug_recurrent_mem_tr__sliding_local_dilated__prompt_kernel(A_x, A_mem0, A_Wq, A_Wk, A_Wv, A_Wo, A_seg_len, B_x, B_wqkv, B_wo):
    del B_x
    B, S, D = A_x.shape
    M = A_mem0.shape[1]
    _, H, DH = A_Wq.shape
    SEG = A_seg_len
    HD = H * DH
    x = A_x.reshape(S, D)
    mem0 = A_mem0.reshape(M, D)
    wq = jnp.transpose(A_Wq, (1, 2, 0)).reshape(HD, D)
    wk = jnp.transpose(A_Wk, (1, 2, 0)).reshape(HD, D)
    wv = jnp.transpose(A_Wv, (1, 2, 0)).reshape(HD, D)
    wo = A_Wo.reshape(HD, D)
    R2 = 2 * M + 2 * SEG
    kern = functools.partial(_kernel, S=S, D=D, H=H, DH=DH, M=M, SEG=SEG, BH=32, BW=8, BDIL=2)
    out = pl.pallas_call(
        kern,
        out_shape=jax.ShapeDtypeStruct((S, D), BF16),
        scratch_shapes=[
            pltpu.VMEM((S + 6 * SEG, D), BF16),
            pltpu.VMEM((2, R2, D), BF16),
            pltpu.VMEM((R2, HD), BF16),
            pltpu.VMEM((R2, HD), BF16),
            pltpu.VMEM((R2, HD), BF16),
            pltpu.VMEM((R2, HD), BF16),
            pltpu.VMEM((D, 3 * D), BF16),
            pltpu.VMEM((D, D), BF16),
            pltpu.VMEM((2, 16 + SEG, D), F32),
            pltpu.VMEM((2, 16 + SEG, D), F32),
        ],
        compiler_params=pltpu.CompilerParams(vmem_limit_bytes=100 * 2**20),
    )(x, mem0, wq, wk, wv, wo, B_wqkv, B_wo)
    return out.reshape(B, S, D)
```

```python
import functools
import jax
import jax.numpy as jnp
from jax import lax
from jax.experimental import pallas as pl
from jax.experimental.pallas import tpu as pltpu

F32 = jnp.float32
BF16 = jnp.bfloat16
NT_DIMS = (((1,), (1,)), ((), ()))
NEG = -1e9
EPS = 1e-5


def _ln(xf):
    m = jnp.mean(xf, axis=-1, keepdims=True)
    d = xf - m
    v = jnp.mean(d * d, axis=-1, keepdims=True)
    return d * lax.rsqrt(v + EPS)


def _dot(a, b):
    return jnp.dot(a, b, preferred_element_type=F32)


def _dot_nt(a, b):
    return lax.dot_general(a, b, NT_DIMS, preferred_element_type=F32)


def _dot_qk(a, b):
    return lax.dot_general(a, b, NT_DIMS, preferred_element_type=F32)


def _dot_pv(a, b):
    return jnp.dot(a, b, preferred_element_type=F32)


def _dot_out(a, b):
    return jnp.dot(a, b, preferred_element_type=F32)


def _dot_bo(a, b):
    return jnp.dot(a, b, preferred_element_type=F32)


def _dot_bqkv(a, b):
    return jnp.dot(a, b, preferred_element_type=F32)


def _kernel(x_ref, mem0_ref, wq_ref, wk_ref, wv_ref, wo_ref, bw_ref, bo_ref, out_ref,
            r_ref, h_ref, o_ref, bwp_ref, bop_ref, qb_ref, kb_ref, vb_ref, acc_ref,
            *, S, D, H, DH, M, SEG, BH, BW, BDIL):
    NS = S // SEG
    NP = H // 2
    PW = 2 * DH
    R2 = 2 * M + 2 * SEG
    PAD = 3
    BDH = D // BH
    HALO = 16

    rr = lax.broadcasted_iota(jnp.int32, (D, D), 0)
    cc = lax.broadcasted_iota(jnp.int32, (D, D), 1)
    src_of_c = (cc % BH) * BDH + cc // BH
    perm = jnp.where(rr == src_of_c, 1.0, 0.0).astype(BF16)
    src_of_r = (rr % BH) * BDH + rr // BH
    permT = jnp.where(cc == src_of_r, 1.0, 0.0).astype(BF16)
    for i in range(3):
        bwp_ref[:, i * D:(i + 1) * D] = _dot(bw_ref[:, i * D:(i + 1) * D], perm).astype(BF16)
    bop_ref[...] = _dot(permT, bo_ref[...]).astype(BF16)

    r_ref[0:PAD * SEG, :] = jnp.zeros((PAD * SEG, D), BF16)
    r_ref[(PAD + NS) * SEG:(2 * PAD + NS) * SEG, :] = jnp.zeros((PAD * SEG, D), BF16)
    r_ref[PAD * SEG:(PAD + NS) * SEG, :] = x_ref[...]
    qb_ref[...] = jnp.zeros(qb_ref.shape, F32)
    kb_ref[...] = jnp.zeros(kb_ref.shape, F32)
    vb_ref[...] = jnp.zeros(vb_ref.shape, F32)

    mem0 = mem0_ref[...].astype(F32)
    mem00 = jnp.concatenate([mem0, mem0], axis=0)
    h_ref[0, 0:2 * M, :] = mem00.astype(BF16)
    h_ref[0, 2 * M:2 * M + SEG, :] = _ln(x_ref[0:SEG, :].astype(F32)).astype(BF16)
    h_ref[0, 2 * M + SEG:R2, :] = jnp.zeros((SEG, D), BF16)

    a_scale = DH ** -0.5
    b_scale = BDH ** -0.5

    def seg(i):
        return pl.ds(pl.multiple_of((i + PAD) * SEG, SEG), SEG)

    NT = D // 128

    def b_local_attn(t):
        obs = []
        for l, sidx in enumerate((t - 1, t - 3)):
            pos = lax.broadcasted_iota(jnp.int32, (SEG, 128), 0) + sidx * SEG
            logits = []
            for w in range(BW):
                r0 = HALO - BDIL * w
                a = None
                for c in range(NT):
                    pr = qb_ref[l, c] * kb_ref[l, c, r0:r0 + SEG, :]
                    a = pr if a is None else a + pr
                a = a + pltpu.roll(a, 64, 1)
                a = a + pltpu.roll(a, 32, 1)
                logits.append(jnp.where(pos >= BDIL * w, a, NEG))
            mx = logits[0]
            for w in range(1, BW):
                mx = jnp.maximum(mx, logits[w])
            es = [jnp.exp(a - mx) for a in logits]
            sm = es[0]
            for w in range(1, BW):
                sm = sm + es[w]
            inv = 1.0 / sm
            aws = [e * inv for e in es]
            tiles = []
            for c in range(NT):
                ob = None
                for w in range(BW):
                    r0 = HALO - BDIL * w
                    term = aws[w] * vb_ref[l, c, r0:r0 + SEG, :]
                    ob = term if ob is None else ob + term
                tiles.append(ob)
            obs.append(jnp.concatenate(tiles, axis=1))
        return jnp.concatenate(obs, axis=0).astype(BF16)

    def b_out(t, ob):
        bout = _dot_bo(ob, bop_ref[...])
        x2 = (r_ref[seg(t - 1), :].astype(F32) + bout[0:SEG]).astype(BF16)
        r_ref[seg(t - 1), :] = x2
        r_ref[seg(t - 3), :] = (r_ref[seg(t - 3), :].astype(F32) + bout[SEG:2 * SEG]).astype(BF16)
        return x2

    def step(t, _):
        slot = lax.rem(t, 2)
        nslot = 1 - slot
        hrows = h_ref[slot]

        NK = 2 * M + 2 * SEG + 2 * M
        ri = lax.broadcasted_iota(jnp.int32, (R2, NK), 0)
        ci = lax.broadcasted_iota(jnp.int32, (R2, NK), 1)
        def layer(i):
            return jnp.where(i < M, 0, jnp.where(i < 2 * M, 1, jnp.where(i < 2 * M + SEG, 0, 1)))
        def allowed(kidx, kvalid):
            return kvalid & (layer(ri) == layer(kidx)) & ((ri < 2 * M) | (kidx < 2 * M) | (ri >= kidx))
        T1, T3, T4 = 2 * M, 2 * M + SEG, 2 * M + 2 * SEG
        mask0 = allowed(ci, ci < T4)
        nat1 = jnp.where(ci < T3, ci - T1 + T3, jnp.where(ci < T4, ci - T3 + T1, ci - T4))
        mask1 = allowed(nat1, ci >= T1)
        lo32 = jnp.where(lax.broadcasted_iota(jnp.int32, (R2 // 2, 128), 1) < 64,
                         jnp.int32(-1), jnp.int32(0))

        def split_lo_hi(z):
            zi = pltpu.bitcast(z, jnp.int32)
            return pltpu.bitcast(zi & lo32, BF16), pltpu.bitcast(zi & ~lo32, BF16)

        def b_weights(z):
            zl, zh = split_lo_hi(z)
            w1 = jnp.concatenate([zl[0:T3], zh[T1:T3], zh[0:T1]], axis=0)
            w3 = jnp.concatenate([zl[0:T1], zh[T3:T4], zl[T3:T4], zh[0:T1]], axis=0)
            return w1, w3

        def h0_rows(z):
            return jnp.concatenate([z, z[0:T1]], axis=0)

        def h1_rows(z):
            return jnp.concatenate([z[0:T1], z[T3:T4], z[T1:T3], z[0:T1]], axis=0)

        def l1_rows(z):
            return z[0:T3]

        def l3_rows(z):
            return jnp.concatenate([z[0:T1], z[T3:T4]], axis=0)

        def merge_rows(y1, y3):
            return jnp.concatenate([y1[0:M], y3[M:T1], y1[T1:T3], y3[T1:T3]], axis=0)

        def proj(w_ref, p):
            c0 = p * PW
            return _dot_nt(hrows, w_ref[c0:c0 + PW, :]).astype(BF16)

        def qk(q, k):
            qA, qB, qC = q[:, 0:128], q[:, 128:256], q[:, 256:384]
            kw1, kw3 = b_weights(k[:, 128:256])
            sa = _dot_qk(qA, h0_rows(k[:, 0:128]))
            sc = _dot_qk(qC, h1_rows(k[:, 256:384]))
            x1 = _dot_qk(l1_rows(qB), kw1)
            x3 = _dot_qk(l3_rows(qB), kw3)
            x = merge_rows(x1, x3)
            return sa + x, sc + x

        def softmax(s, mask):
            s = jnp.where(mask, s * a_scale, NEG)
            mx = jnp.max(s, axis=-1, keepdims=True)
            e = jnp.exp(s - mx)
            sm = jnp.sum(e, axis=-1, keepdims=True)
            return e * (1.0 / sm)

        def pv(p, s0, s1, v):
            c0 = p * PW
            p0 = softmax(s0, mask0)
            p1 = softmax(s1, mask1)
            pm = (p0 + p1).astype(BF16)
            vw1, vw3 = b_weights(v[:, 128:256])
            oa = _dot_pv(p0.astype(BF16), h0_rows(v[:, 0:128]))
            oc = _dot_pv(p1.astype(BF16), h1_rows(v[:, 256:384]))
            y1 = _dot_pv(l1_rows(pm), vw1)
            y3 = _dot_pv(l3_rows(pm), vw3)
            o_ref[:, c0:c0 + 128] = oa.astype(BF16)
            o_ref[:, c0 + 128:c0 + 256] = merge_rows(y1, y3).astype(BF16)
            o_ref[:, c0 + 256:c0 + 384] = oc.astype(BF16)

        ob = b_local_attn(t)

        q, k, v = proj(wq_ref, 0), proj(wk_ref, 0), proj(wv_ref, 0)
        for p in range(1, NP):
            s0, s1 = qk(q, k)
            qn = proj(wq_ref, p)
            kn = proj(wk_ref, p)
            pv(p - 1, s0, s1, v)
            v = proj(wv_ref, p)
            q, k = qn, kn
        s0, s1 = qk(q, k)
        KS1 = (NP // 2) * PW
        KS2 = (NP - 1) * PW
        acc_ref[...] = _dot_out(o_ref[:, 0:KS1], wo_ref[0:KS1, :])
        pv(NP - 1, s0, s1, v)
        a2 = _dot_out(o_ref[:, KS1:], wo_ref[KS1:, :])
        aout = acc_ref[...] + a2

        x1 = (r_ref[seg(t), :].astype(F32) + aout[2 * M:2 * M + SEG]).astype(BF16)
        x3 = (r_ref[seg(t - 2), :].astype(F32) + aout[2 * M + SEG:R2]).astype(BF16)
        r_ref[seg(t), :] = x1
        r_ref[seg(t - 2), :] = x3
        mrow = lax.broadcasted_iota(jnp.int32, (2 * M, D), 0)
        keep = (mrow < M) | (t >= 2)
        h_ref[nslot, 0:2 * M, :] = jnp.where(keep, aout[0:2 * M], mem00).astype(BF16)
        h_ref[nslot, 2 * M:2 * M + SEG, :] = _ln(r_ref[seg(t + 1), :].astype(F32)).astype(BF16)

        x2 = b_out(t, ob)
        h_ref[nslot, 2 * M + SEG:R2, :] = _ln(x2.astype(F32)).astype(BF16)

        hb = jnp.concatenate([_ln(x1.astype(F32)), _ln(x3.astype(F32))], axis=0).astype(BF16)
        qkv = _dot_bqkv(hb, bwp_ref[...])
        for l in range(2):
            rows = slice(l * SEG, (l + 1) * SEG)
            for c in range(NT):
                cs = slice(c * 128, (c + 1) * 128)
                qb_ref[l, c] = qkv[rows, cs] * b_scale
                kb_ref[l, c, 0:HALO, :] = kb_ref[l, c, SEG:SEG + HALO, :]
                vb_ref[l, c, 0:HALO, :] = vb_ref[l, c, SEG:SEG + HALO, :]
                kb_ref[l, c, HALO:HALO + SEG, :] = qkv[rows, D + c * 128:D + (c + 1) * 128]
                vb_ref[l, c, HALO:HALO + SEG, :] = qkv[rows, 2 * D + c * 128:2 * D + (c + 1) * 128]
        return 0

    lax.fori_loop(0, NS + 2, step, 0)
    b_out(NS + 2, b_local_attn(NS + 2))
    out_ref[...] = r_ref[PAD * SEG:(PAD + NS) * SEG, :]


@functools.partial(jax.jit, static_argnames=("A_seg_len",))
def pallas_interleave_layers__memory_aug_recurrent_mem_tr__sliding_local_dilated__prompt_kernel(A_x, A_mem0, A_Wq, A_Wk, A_Wv, A_Wo, A_seg_len, B_x, B_wqkv, B_wo):
    del B_x
    B, S, D = A_x.shape
    M = A_mem0.shape[1]
    _, H, DH = A_Wq.shape
    SEG = A_seg_len
    HD = H * DH
    x = A_x.reshape(S, D)
    mem0 = A_mem0.reshape(M, D)
    wq = jnp.transpose(A_Wq, (1, 2, 0)).reshape(HD, D)
    wk = jnp.transpose(A_Wk, (1, 2, 0)).reshape(HD, D)
    wv = jnp.transpose(A_Wv, (1, 2, 0)).reshape(HD, D)
    wo = A_Wo.reshape(HD, D)
    R2 = 2 * M + 2 * SEG
    kern = functools.partial(_kernel, S=S, D=D, H=H, DH=DH, M=M, SEG=SEG, BH=32, BW=8, BDIL=2)
    out = pl.pallas_call(
        kern,
        out_shape=jax.ShapeDtypeStruct((S, D), BF16),
        scratch_shapes=[
            pltpu.VMEM((S + 6 * SEG, D), BF16),
            pltpu.VMEM((2, R2, D), BF16),
            pltpu.VMEM((R2, HD), BF16),
            pltpu.VMEM((D, 3 * D), BF16),
            pltpu.VMEM((D, D), BF16),
            pltpu.VMEM((2, D // 128, SEG, 128), F32),
            pltpu.VMEM((2, D // 128, 16 + SEG, 128), F32),
            pltpu.VMEM((2, D // 128, 16 + SEG, 128), F32),
            pltpu.VMEM((R2, D), F32),
        ],
        compiler_params=pltpu.CompilerParams(vmem_limit_bytes=100 * 2**20),
    )(x, mem0, wq, wk, wv, wo, B_wqkv, B_wo)
    return out.reshape(B, S, D)
```

```python
import functools
import jax
import jax.numpy as jnp
from jax import lax
from jax.experimental import pallas as pl
from jax.experimental.pallas import tpu as pltpu

F32 = jnp.float32
BF16 = jnp.bfloat16
I32 = jnp.int32
NT_DIMS = (((1,), (1,)), ((), ()))
NEG = -1e9
EPS = 1e-5


def _ln(xf):
    m = jnp.mean(xf, axis=-1, keepdims=True)
    d = xf - m
    v = jnp.mean(d * d, axis=-1, keepdims=True)
    return d * lax.rsqrt(v + EPS)


def _dot(a, b):
    return jnp.dot(a, b, preferred_element_type=F32)


def _dot_nt(a, b):
    return lax.dot_general(a, b, NT_DIMS, preferred_element_type=F32)


def _dot_qk(a, b):
    return lax.dot_general(a, b, NT_DIMS, preferred_element_type=F32)


def _dot_pv(a, b):
    return jnp.dot(a, b, preferred_element_type=F32)


def _dot_out(a, b):
    return jnp.dot(a, b, preferred_element_type=F32)


def _dot_bo(a, b):
    return jnp.dot(a, b, preferred_element_type=F32)


def _dot_bqkv(a, b):
    return jnp.dot(a, b, preferred_element_type=F32)


def _kernel(x_hbm, mem0_ref, wq_hbm, wk_hbm, wv_hbm, wo_hbm, bw_hbm, bo_hbm, out_ref,
            r_ref, h_ref, o_ref, bwp_ref, bop_ref, qb_ref, kb_ref, vb_ref, acc_ref,
            x_ref, wq_ref, wk_ref, wv_ref, wo_ref, bw_ref, bo_ref, sems,
            *, S, D, H, DH, M, SEG, BH, BW, BDIL):
    NS = S // SEG
    NP = H // 2
    PW = 2 * DH
    R2 = 2 * M + 2 * SEG
    PAD = 3
    BDH = D // BH
    HALO = 16
    NT = D // 128
    T1, T3, T4 = 2 * M, 2 * M + SEG, 2 * M + 2 * SEG
    NK = T4 + T1
    a_scale = DH ** -0.5
    b_scale = BDH ** -0.5

    cp_bw = pltpu.make_async_copy(bw_hbm, bw_ref, sems.at[0])
    cp_bo = pltpu.make_async_copy(bo_hbm, bo_ref, sems.at[1])
    cp_x = pltpu.make_async_copy(x_hbm, x_ref, sems.at[2])
    cp_q = pltpu.make_async_copy(wq_hbm, wq_ref, sems.at[3])
    cp_k = pltpu.make_async_copy(wk_hbm, wk_ref, sems.at[4])
    cp_v = pltpu.make_async_copy(wv_hbm, wv_ref, sems.at[5])
    cp_o = pltpu.make_async_copy(wo_hbm, wo_ref, sems.at[6])
    for cp in (cp_bw, cp_bo, cp_x, cp_q, cp_k, cp_v, cp_o):
        cp.start()
    cp_bw.wait()
    cp_bo.wait()

    rr = lax.broadcasted_iota(I32, (D, D), 0)
    cc = lax.broadcasted_iota(I32, (D, D), 1)
    src_of_c = (cc % BH) * BDH + cc // BH
    perm = jnp.where(rr == src_of_c, 1.0, 0.0).astype(BF16)
    src_of_r = (rr % BH) * BDH + rr // BH
    permT = jnp.where(cc == src_of_r, 1.0, 0.0).astype(BF16)
    for i in range(3):
        bwp_ref[:, i * D:(i + 1) * D] = _dot(bw_ref[:, i * D:(i + 1) * D], perm).astype(BF16)
    bop_ref[...] = _dot(permT, bo_ref[...]).astype(BF16)

    r_ref[0:PAD * SEG, :] = jnp.zeros((PAD * SEG, D), BF16)
    r_ref[(PAD + NS) * SEG:(2 * PAD + NS) * SEG, :] = jnp.zeros((PAD * SEG, D), BF16)
    cp_x.wait()
    r_ref[PAD * SEG:(PAD + NS) * SEG, :] = x_ref[...]
    qb_ref[...] = jnp.zeros(qb_ref.shape, F32)
    kb_ref[...] = jnp.zeros(kb_ref.shape, F32)
    vb_ref[...] = jnp.zeros(vb_ref.shape, F32)

    mem0 = mem0_ref[...].astype(F32)
    mem00 = jnp.concatenate([mem0, mem0], axis=0)
    h_ref[0, 0:T1, :] = mem00.astype(BF16)
    h_ref[0, T1:T3, :] = _ln(x_ref[0:SEG, :].astype(F32)).astype(BF16)
    h_ref[0, T3:T4, :] = jnp.zeros((SEG, D), BF16)

    def seg(i):
        return pl.ds(pl.multiple_of((i + PAD) * SEG, SEG), SEG)

    def b_local_attn(t):
        obs = []
        for l, sidx in enumerate((t - 1, t - 3)):
            pos = lax.broadcasted_iota(I32, (SEG, 128), 0) + sidx * SEG
            logits = []
            for w in range(BW):
                r0 = HALO - BDIL * w
                a = None
                for c in range(NT):
                    pr = qb_ref[l, c] * kb_ref[l, c, r0:r0 + SEG, :]
                    a = pr if a is None else a + pr
                a = a + pltpu.roll(a, 64, 1)
                a = a + pltpu.roll(a, 32, 1)
                logits.append(jnp.where(pos >= BDIL * w, a, NEG))
            mx = logits[0]
            for w in range(1, BW):
                mx = jnp.maximum(mx, logits[w])
            es = [jnp.exp(a - mx) for a in logits]
            sm = es[0]
            for w in range(1, BW):
                sm = sm + es[w]
            inv = 1.0 / sm
            aws = [e * inv for e in es]
            tiles = []
            for c in range(NT):
                ob = None
                for w in range(BW):
                    r0 = HALO - BDIL * w
                    term = aws[w] * vb_ref[l, c, r0:r0 + SEG, :]
                    ob = term if ob is None else ob + term
                tiles.append(ob)
            obs.append(jnp.concatenate(tiles, axis=1))
        return jnp.concatenate(obs, axis=0).astype(BF16)

    def b_out(t, ob):
        bout = _dot_bo(ob, bop_ref[...])
        x2 = (r_ref[seg(t - 1), :].astype(F32) + bout[0:SEG]).astype(BF16)
        r_ref[seg(t - 1), :] = x2
        r_ref[seg(t - 3), :] = (r_ref[seg(t - 3), :].astype(F32) + bout[SEG:2 * SEG]).astype(BF16)
        return x2

    def b_qkv(xa, xb):
        hb = jnp.concatenate([_ln(xa.astype(F32)), _ln(xb.astype(F32))], axis=0).astype(BF16)
        qkv = _dot_bqkv(hb, bwp_ref[...])
        for l in range(2):
            rows = slice(l * SEG, (l + 1) * SEG)
            for c in range(NT):
                cs = slice(c * 128, (c + 1) * 128)
                qb_ref[l, c] = qkv[rows, cs] * b_scale
                kb_ref[l, c, 0:HALO, :] = kb_ref[l, c, SEG:SEG + HALO, :]
                vb_ref[l, c, 0:HALO, :] = vb_ref[l, c, SEG:SEG + HALO, :]
                kb_ref[l, c, HALO:HALO + SEG, :] = qkv[rows, D + c * 128:D + (c + 1) * 128]
                vb_ref[l, c, HALO:HALO + SEG, :] = qkv[rows, 2 * D + c * 128:2 * D + (c + 1) * 128]

    def softmax(s, mask):
        s = jnp.where(mask, s * a_scale, NEG)
        mx = jnp.max(s, axis=-1, keepdims=True)
        e = jnp.exp(s - mx)
        sm = jnp.sum(e, axis=-1, keepdims=True)
        return e * (1.0 / sm)

    def split_lo_hi(z):
        rows = z.shape[0]
        lo32 = jnp.where(lax.broadcasted_iota(I32, (rows // 2, 128), 1) < 64, I32(-1), I32(0))
        zi = pltpu.bitcast(z, I32)
        return pltpu.bitcast(zi & lo32, BF16), pltpu.bitcast(zi & ~lo32, BF16)

    def step(t, full):
        slot = lax.rem(t, 2)
        nslot = 1 - slot
        if full:
            RW = R2
            hrows = h_ref[slot]
        else:
            RW = T3
            lay = jnp.where(t < 2, 0, 1)
            hrows = jnp.concatenate(
                [h_ref[slot, 0:T1, :],
                 h_ref[slot, pl.ds(pl.multiple_of(T1 + lay * SEG, 16), SEG), :]], axis=0)

        ri = lax.broadcasted_iota(I32, (RW, NK), 0)
        ci = lax.broadcasted_iota(I32, (RW, NK), 1)
        if full:
            def layer(i):
                return jnp.where(i < M, 0, jnp.where(i < T1, 1, jnp.where(i < T3, 0, 1)))
            def allowed(kidx, kvalid):
                return kvalid & (layer(ri) == layer(kidx)) & ((ri < T1) | (kidx < T1) | (ri >= kidx))
            mask0 = allowed(ci, ci < T4)
            nat1 = jnp.where(ci < T3, ci - T1 + T3, jnp.where(ci < T4, ci - T3 + T1, ci - T4))
            mask1 = allowed(nat1, ci >= T1)
        else:
            def allowed(kidx, kvalid):
                kok = kvalid & ((kidx >= T1) | (kidx // M == lay))
                return kok & ((ri < T1) | (kidx < T1) | (ri >= kidx))
            mask0 = allowed(ci, ci < T3)
            nat1 = jnp.where(ci < T4, ci - T3 + T1, ci - T4)
            mask1 = allowed(nat1, ci >= T3)

        def proj(w_ref, p):
            c0 = p * PW
            return _dot_nt(hrows, w_ref[c0:c0 + PW, :]).astype(BF16)

        if full:
            def b_weights(z):
                zl, zh = split_lo_hi(z)
                w1 = jnp.concatenate([zl[0:T3], zh[T1:T3], zh[0:T1]], axis=0)
                w3 = jnp.concatenate([zl[0:T1], zh[T3:T4], zl[T3:T4], zh[0:T1]], axis=0)
                return w1, w3

            def h0_rows(z):
                return jnp.concatenate([z, z[0:T1]], axis=0)

            def h1_rows(z):
                return jnp.concatenate([z[0:T1], z[T3:T4], z[T1:T3], z[0:T1]], axis=0)

            def shared(dot, lhs, ws):
                y1 = dot(lhs[0:T3], ws[0])
                y3 = dot(jnp.concatenate([lhs[0:T1], lhs[T3:T4]], axis=0), ws[1])
                return jnp.concatenate([y1[0:M], y3[M:T1], y1[T1:T3], y3[T1:T3]], axis=0)
        else:
            def b_weights(z):
                zl, zh = split_lo_hi(z)
                return (jnp.concatenate([zl, zh[T1:T3], zh[0:T1]], axis=0),)

            def h0_rows(z):
                return jnp.concatenate([z, z], axis=0)

            def h1_rows(z):
                return jnp.concatenate([z, z[T1:T3], z[0:T1]], axis=0)

            def shared(dot, lhs, ws):
                return dot(lhs, ws[0])

        def qk(q, k):
            qA, qB, qC = q[:, 0:128], q[:, 128:256], q[:, 256:384]
            sa = _dot_qk(qA, h0_rows(k[:, 0:128]))
            sc = _dot_qk(qC, h1_rows(k[:, 256:384]))
            x = shared(_dot_qk, qB, b_weights(k[:, 128:256]))
            return sa + x, sc + x

        def pv(p, s0, s1, v):
            c0 = p * PW
            p0 = softmax(s0, mask0)
            p1 = softmax(s1, mask1)
            pm = (p0 + p1).astype(BF16)
            oa = _dot_pv(p0.astype(BF16), h0_rows(v[:, 0:128]))
            oc = _dot_pv(p1.astype(BF16), h1_rows(v[:, 256:384]))
            ob_ = shared(_dot_pv, pm, b_weights(v[:, 128:256]))
            o_ref[0:RW, c0:c0 + 128] = oa.astype(BF16)
            o_ref[0:RW, c0 + 128:c0 + 256] = ob_.astype(BF16)
            o_ref[0:RW, c0 + 256:c0 + 384] = oc.astype(BF16)

        ob = b_local_attn(t)

        q, k, v = proj(wq_ref, 0), proj(wk_ref, 0), proj(wv_ref, 0)
        for p in range(1, NP):
            s0, s1 = qk(q, k)
            qn = proj(wq_ref, p)
            kn = proj(wk_ref, p)
            pv(p - 1, s0, s1, v)
            v = proj(wv_ref, p)
            q, k = qn, kn
        s0, s1 = qk(q, k)
        if not full:
            @pl.when(t == 0)
            def _():
                cp_o.wait()
        KS1 = (NP // 2) * PW
        acc_ref[0:RW] = _dot_out(o_ref[0:RW, 0:KS1], wo_ref[0:KS1, :])
        pv(NP - 1, s0, s1, v)
        aout = acc_ref[0:RW] + _dot_out(o_ref[0:RW, KS1:], wo_ref[KS1:, :])

        if full:
            x1 = (r_ref[seg(t), :].astype(F32) + aout[T1:T3]).astype(BF16)
            x3 = (r_ref[seg(t - 2), :].astype(F32) + aout[T3:T4]).astype(BF16)
            r_ref[seg(t), :] = x1
            r_ref[seg(t - 2), :] = x3
        else:
            sg = seg(t - 2 * lay)
            r_ref[sg, :] = (r_ref[sg, :].astype(F32) + aout[T1:T3]).astype(BF16)
            x1 = r_ref[seg(t), :]
            x3 = r_ref[seg(t - 2), :]
        mrow = lax.broadcasted_iota(I32, (T1, D), 0)
        keep = (mrow < M) | (t >= 2)
        h_ref[nslot, 0:T1, :] = jnp.where(keep, aout[0:T1], mem00).astype(BF16)
        h_ref[nslot, T1:T3, :] = _ln(r_ref[seg(t + 1), :].astype(F32)).astype(BF16)

        x2 = b_out(t, ob)
        h_ref[nslot, T3:T4, :] = _ln(x2.astype(F32)).astype(BF16)
        b_qkv(x1, x3)

    def body(t, _):
        edge = (t < 2) | (t >= NS)

        @pl.when(edge)
        def _():
            step(t, False)

        @pl.when(jnp.logical_not(edge))
        def _():
            step(t, True)
        return 0

    cp_q.wait()
    cp_k.wait()
    cp_v.wait()
    lax.fori_loop(0, NS + 2, body, 0)
    b_out(NS + 2, b_local_attn(NS + 2))
    out_ref[...] = r_ref[PAD * SEG:(PAD + NS) * SEG, :]


@functools.partial(jax.jit, static_argnames=("A_seg_len",))
def pallas_interleave_layers__memory_aug_recurrent_mem_tr__sliding_local_dilated__prompt_kernel(A_x, A_mem0, A_Wq, A_Wk, A_Wv, A_Wo, A_seg_len, B_x, B_wqkv, B_wo):
    del B_x
    B, S, D = A_x.shape
    M = A_mem0.shape[1]
    _, H, DH = A_Wq.shape
    SEG = A_seg_len
    HD = H * DH
    x = A_x.reshape(S, D)
    mem0 = A_mem0.reshape(M, D)
    wq = jnp.transpose(A_Wq, (1, 2, 0)).reshape(HD, D)
    wk = jnp.transpose(A_Wk, (1, 2, 0)).reshape(HD, D)
    wv = jnp.transpose(A_Wv, (1, 2, 0)).reshape(HD, D)
    wo = A_Wo.reshape(HD, D)
    R2 = 2 * M + 2 * SEG
    kern = functools.partial(_kernel, S=S, D=D, H=H, DH=DH, M=M, SEG=SEG, BH=32, BW=8, BDIL=2)
    out = pl.pallas_call(
        kern,
        out_shape=jax.ShapeDtypeStruct((S, D), BF16),
        in_specs=[pl.BlockSpec(memory_space=pl.ANY), pl.BlockSpec(memory_space=pltpu.VMEM)]
        + [pl.BlockSpec(memory_space=pl.ANY)] * 6,
        scratch_shapes=[
            pltpu.VMEM((S + 6 * SEG, D), BF16),
            pltpu.VMEM((2, R2, D), BF16),
            pltpu.VMEM((R2, HD), BF16),
            pltpu.VMEM((D, 3 * D), BF16),
            pltpu.VMEM((D, D), BF16),
            pltpu.VMEM((2, D // 128, SEG, 128), F32),
            pltpu.VMEM((2, D // 128, 16 + SEG, 128), F32),
            pltpu.VMEM((2, D // 128, 16 + SEG, 128), F32),
            pltpu.VMEM((R2, D), F32),
            pltpu.VMEM((S, D), BF16),
            pltpu.VMEM((HD, D), BF16),
            pltpu.VMEM((HD, D), BF16),
            pltpu.VMEM((HD, D), BF16),
            pltpu.VMEM((HD, D), BF16),
            pltpu.VMEM((D, 3 * D), BF16),
            pltpu.VMEM((D, D), BF16),
            pltpu.SemaphoreType.DMA((8,)),
        ],
        compiler_params=pltpu.CompilerParams(vmem_limit_bytes=100 * 2**20),
    )(x, mem0, wq, wk, wv, wo, B_wqkv, B_wo)
    return out.reshape(B, S, D)
```

```python
import functools
import jax
import jax.numpy as jnp
from jax import lax
from jax.experimental import pallas as pl
from jax.experimental.pallas import tpu as pltpu

F32 = jnp.float32
BF16 = jnp.bfloat16
I32 = jnp.int32
NT_DIMS = (((1,), (1,)), ((), ()))
NEG = -1e9
EPS = 1e-5


def _ln(xf):
    m = jnp.mean(xf, axis=-1, keepdims=True)
    d = xf - m
    v = jnp.mean(d * d, axis=-1, keepdims=True)
    return d * lax.rsqrt(v + EPS)


def _dot(a, b):
    return jnp.dot(a, b, preferred_element_type=F32)


def _dot_nt(a, b):
    return lax.dot_general(a, b, NT_DIMS, preferred_element_type=F32)


def _dot_nn(a, b):
    return jnp.dot(a, b, preferred_element_type=F32)


def _dot_qk(a, b):
    return lax.dot_general(a, b, NT_DIMS, preferred_element_type=F32)


def _dot_pv(a, b):
    return jnp.dot(a, b, preferred_element_type=F32)


def _dot_out(a, b):
    return jnp.dot(a, b, preferred_element_type=F32)


def _dot_bo(a, b):
    return jnp.dot(a, b, preferred_element_type=F32)


def _dot_bqkv(a, b):
    return jnp.dot(a, b, preferred_element_type=F32)


def _kernel(x_hbm, mem0_ref, wq_hbm, wk_hbm, wv_hbm, wo_hbm, bw_hbm, bo_hbm, out_hbm,
            r_ref, h_ref, o_ref, bwp_ref, bop_ref, qb_ref, kb_ref, vb_ref, acc_ref,
            sq_ref, sk_ref, sv_ref, wq_ref, wk_ref, wv_ref, wo_ref, bw_ref, bo_ref,
            hpre_ref, pq_ref, pk_ref, pv_ref, sems, psems,
            *, S, D, H, DH, M, SEG, BH, BW, BDIL, NPRE):
    NS = S // SEG
    NP = H // 2
    PW = 2 * DH
    R2 = 2 * M + 2 * SEG
    PAD = 3
    BDH = D // BH
    HALO = 16
    NT = D // 128
    T1, T3, T4 = 2 * M, 2 * M + SEG, 2 * M + 2 * SEG
    NK = T4 + T1
    a_scale = DH ** -0.5
    b_scale = BDH ** -0.5
    AHEAD = 8
    XH = (NPRE + 1) * SEG

    cp_bw = pltpu.make_async_copy(bw_hbm, bw_ref, sems.at[0])
    cp_bo = pltpu.make_async_copy(bo_hbm, bo_ref, sems.at[1])
    cp_xh = pltpu.make_async_copy(x_hbm.at[0:XH], r_ref.at[PAD * SEG:PAD * SEG + XH], sems.at[2])
    cp_xt = pltpu.make_async_copy(x_hbm.at[XH:S], r_ref.at[PAD * SEG + XH:PAD * SEG + S], sems.at[3])
    cp_o = pltpu.make_async_copy(wo_hbm, wo_ref, sems.at[4])

    def pair_copies(p):
        rows = pl.ds(pl.multiple_of(p * PW, PW), PW)
        return [pltpu.make_async_copy(w.at[rows], s.at[rows], psems.at[p])
                for w, s in ((wq_hbm, sq_ref), (wk_hbm, sk_ref), (wv_hbm, sv_ref))]

    cp_bw.start()
    cp_bo.start()
    cp_xh.start()
    cp_bw.wait()
    cp_bo.wait()
    for p in range(AHEAD):
        for cp in pair_copies(p):
            cp.start()

    rr = lax.broadcasted_iota(I32, (D, D), 0)
    cc = lax.broadcasted_iota(I32, (D, D), 1)
    src_of_c = (cc % BH) * BDH + cc // BH
    perm = jnp.where(rr == src_of_c, 1.0, 0.0).astype(BF16)
    src_of_r = (rr % BH) * BDH + rr // BH
    permT = jnp.where(cc == src_of_r, 1.0, 0.0).astype(BF16)
    for i in range(3):
        bwp_ref[:, i * D:(i + 1) * D] = _dot(bw_ref[:, i * D:(i + 1) * D], perm).astype(BF16)
    bop_ref[...] = _dot(permT, bo_ref[...]).astype(BF16)

    r_ref[0:PAD * SEG, :] = jnp.zeros((PAD * SEG, D), BF16)
    r_ref[(PAD + NS) * SEG:(2 * PAD + NS) * SEG, :] = jnp.zeros((PAD * SEG, D), BF16)
    qb_ref[...] = jnp.zeros(qb_ref.shape, F32)
    kb_ref[...] = jnp.zeros(kb_ref.shape, F32)
    vb_ref[...] = jnp.zeros(vb_ref.shape, F32)

    mem0 = mem0_ref[...].astype(F32)
    mem00 = jnp.concatenate([mem0, mem0], axis=0)
    h_ref[0, 0:T1, :] = mem00.astype(BF16)
    cp_xh.wait()
    hpre_ref[...] = _ln(r_ref[PAD * SEG:(PAD + NPRE) * SEG, :].astype(F32)).astype(BF16)

    def pair_prologue(p, _):
        for cp in pair_copies(p):
            cp.wait()

        @pl.when(p + AHEAD < NP)
        def _():
            for cp in pair_copies(p + AHEAD):
                cp.start()

        @pl.when(p + AHEAD == NP)
        def _():
            cp_o.start()
            cp_xt.start()

        rows = pl.ds(pl.multiple_of(p * PW, PW), PW)
        cols = pl.ds(pl.multiple_of(p * PW, 128), PW)
        hp = hpre_ref[...]
        for s_ref, w_ref, p_ref in ((sq_ref, wq_ref, pq_ref), (sk_ref, wk_ref, pk_ref),
                                    (sv_ref, wv_ref, pv_ref)):
            w = s_ref[rows, :]
            p_ref[:, cols] = _dot_nt(hp, w).astype(BF16)
            w_ref[:, cols] = w.T
        return 0

    lax.fori_loop(0, NP, pair_prologue, 0)

    def seg(i):
        return pl.ds(pl.multiple_of((i + PAD) * SEG, SEG), SEG)

    def b_local_attn(t):
        obs = []
        for l, sidx in enumerate((t - 1, t - 3)):
            pos = lax.broadcasted_iota(I32, (SEG, 128), 0) + sidx * SEG
            logits = []
            for w in range(BW):
                r0 = HALO - BDIL * w
                a = None
                for c in range(NT):
                    pr = qb_ref[l, c] * kb_ref[l, c, r0:r0 + SEG, :]
                    a = pr if a is None else a + pr
                a = a + pltpu.roll(a, 64, 1)
                a = a + pltpu.roll(a, 32, 1)
                logits.append(jnp.where(pos >= BDIL * w, a, NEG))
            mx = logits[0]
            for w in range(1, BW):
                mx = jnp.maximum(mx, logits[w])
            es = [jnp.exp(a - mx) for a in logits]
            sm = es[0]
            for w in range(1, BW):
                sm = sm + es[w]
            inv = 1.0 / sm
            aws = [e * inv for e in es]
            tiles = []
            for c in range(NT):
                ob = None
                for w in range(BW):
                    r0 = HALO - BDIL * w
                    term = aws[w] * vb_ref[l, c, r0:r0 + SEG, :]
                    ob = term if ob is None else ob + term
                tiles.append(ob)
            obs.append(jnp.concatenate(tiles, axis=1))
        return jnp.concatenate(obs, axis=0).astype(BF16)

    def b_out(t, ob):
        bout = _dot_bo(ob, bop_ref[...])
        x2 = (r_ref[seg(t - 1), :].astype(F32) + bout[0:SEG]).astype(BF16)
        r_ref[seg(t - 1), :] = x2
        r_ref[seg(t - 3), :] = (r_ref[seg(t - 3), :].astype(F32) + bout[SEG:2 * SEG]).astype(BF16)
        return x2

    def b_qkv(xa, xb):
        hb = jnp.concatenate([_ln(xa.astype(F32)), _ln(xb.astype(F32))], axis=0).astype(BF16)
        qkv = _dot_bqkv(hb, bwp_ref[...])
        for l in range(2):
            rows = slice(l * SEG, (l + 1) * SEG)
            for c in range(NT):
                cs = slice(c * 128, (c + 1) * 128)
                qb_ref[l, c] = qkv[rows, cs] * b_scale
                kb_ref[l, c, 0:HALO, :] = kb_ref[l, c, SEG:SEG + HALO, :]
                vb_ref[l, c, 0:HALO, :] = vb_ref[l, c, SEG:SEG + HALO, :]
                kb_ref[l, c, HALO:HALO + SEG, :] = qkv[rows, D + c * 128:D + (c + 1) * 128]
                vb_ref[l, c, HALO:HALO + SEG, :] = qkv[rows, 2 * D + c * 128:2 * D + (c + 1) * 128]

    def softmax(s, mask):
        s = jnp.where(mask, s * a_scale, NEG)
        mx = jnp.max(s, axis=-1, keepdims=True)
        e = jnp.exp(s - mx)
        sm = jnp.sum(e, axis=-1, keepdims=True)
        return e * (1.0 / sm)

    def split_lo_hi(z):
        rows = z.shape[0]
        lo32 = jnp.where(lax.broadcasted_iota(I32, (rows // 2, 128), 1) < 64, I32(-1), I32(0))
        zi = pltpu.bitcast(z, I32)
        return pltpu.bitcast(zi & lo32, BF16), pltpu.bitcast(zi & ~lo32, BF16)

    def step(t, pass1, pass3, active):
        slot = lax.rem(t, 2)
        nslot = 1 - slot
        full = active is None
        lay = active
        RW = R2 if full else T3
        parts = [h_ref[slot, 0:T1, :]]
        if pass1:
            parts.append(h_ref[slot, T1:T3, :])
        if pass3:
            parts.append(h_ref[slot, T3:T4, :])
        hrows = h_ref[slot] if (pass1 and pass3) else jnp.concatenate(parts, axis=0)

        ri = lax.broadcasted_iota(I32, (RW, NK), 0)
        ci = lax.broadcasted_iota(I32, (RW, NK), 1)
        if full:
            def layer(i):
                return jnp.where(i < M, 0, jnp.where(i < T1, 1, jnp.where(i < T3, 0, 1)))
            def allowed(kidx, kvalid):
                return kvalid & (layer(ri) == layer(kidx)) & ((ri < T1) | (kidx < T1) | (ri >= kidx))
            mask0 = allowed(ci, ci < T4)
            nat1 = jnp.where(ci < T3, ci - T1 + T3, jnp.where(ci < T4, ci - T3 + T1, ci - T4))
            mask1 = allowed(nat1, ci >= T1)
        else:
            def allowed(kidx, kvalid):
                kok = kvalid & ((kidx >= T1) | (kidx // M == lay))
                return kok & ((ri < T1) | (kidx < T1) | (ri >= kidx))
            mask0 = allowed(ci, ci < T3)
            nat1 = jnp.where(ci < T4, ci - T3 + T1, ci - T4)
            mask1 = allowed(nat1, ci >= T3)

        def proj(w_ref, pre_ref, p):
            c0 = p * PW
            y = _dot_nn(hrows, w_ref[:, c0:c0 + PW]).astype(BF16)
            if pass1 or lay == 1:
                return y
            pre = pre_ref[pl.ds(pl.multiple_of(t * SEG, SEG), SEG), c0:c0 + PW]
            if pass3:
                return jnp.concatenate([y[0:T1], pre, y[T1:T3]], axis=0)
            return jnp.concatenate([y, pre], axis=0)

        if full:
            def b_weights(z):
                zl, zh = split_lo_hi(z)
                w1 = jnp.concatenate([zl[0:T3], zh[T1:T3], zh[0:T1]], axis=0)
                w3 = jnp.concatenate([zl[0:T1], zh[T3:T4], zl[T3:T4], zh[0:T1]], axis=0)
                return w1, w3

            def h0_rows(z):
                return jnp.concatenate([z, z[0:T1]], axis=0)

            def h1_rows(z):
                return jnp.concatenate([z[0:T1], z[T3:T4], z[T1:T3], z[0:T1]], axis=0)

            def shared(dot, lhs, ws):
                y1 = dot(lhs[0:T3], ws[0])
                y3 = dot(jnp.concatenate([lhs[0:T1], lhs[T3:T4]], axis=0), ws[1])
                return jnp.concatenate([y1[0:M], y3[M:T1], y1[T1:T3], y3[T1:T3]], axis=0)
        else:
            def b_weights(z):
                zl, zh = split_lo_hi(z)
                return (jnp.concatenate([zl, zh[T1:T3], zh[0:T1]], axis=0),)

            def h0_rows(z):
                return jnp.concatenate([z, z], axis=0)

            def h1_rows(z):
                return jnp.concatenate([z, z[T1:T3], z[0:T1]], axis=0)

            def shared(dot, lhs, ws):
                return dot(lhs, ws[0])

        def qk(q, k):
            qA, qB, qC = q[:, 0:128], q[:, 128:256], q[:, 256:384]
            sa = _dot_qk(qA, h0_rows(k[:, 0:128]))
            sc = _dot_qk(qC, h1_rows(k[:, 256:384]))
            x = shared(_dot_qk, qB, b_weights(k[:, 128:256]))
            return sa + x, sc + x

        def pv(p, s0, s1, v):
            c0 = p * PW
            p0 = softmax(s0, mask0)
            p1 = softmax(s1, mask1)
            pm = (p0 + p1).astype(BF16)
            oa = _dot_pv(p0.astype(BF16), h0_rows(v[:, 0:128]))
            oc = _dot_pv(p1.astype(BF16), h1_rows(v[:, 256:384]))
            ob_ = shared(_dot_pv, pm, b_weights(v[:, 128:256]))
            o_ref[0:RW, c0:c0 + 128] = oa.astype(BF16)
            o_ref[0:RW, c0 + 128:c0 + 256] = ob_.astype(BF16)
            o_ref[0:RW, c0 + 256:c0 + 384] = oc.astype(BF16)

        if not pass1 and not pass3:
            @pl.when(t == 1)
            def _():
                cp_xt.wait()

        ob = b_local_attn(t)

        q, k, v = proj(wq_ref, pq_ref, 0), proj(wk_ref, pk_ref, 0), proj(wv_ref, pv_ref, 0)
        for p in range(1, NP):
            s0, s1 = qk(q, k)
            qn = proj(wq_ref, pq_ref, p)
            kn = proj(wk_ref, pk_ref, p)
            pv(p - 1, s0, s1, v)
            v = proj(wv_ref, pv_ref, p)
            q, k = qn, kn
        s0, s1 = qk(q, k)
        if not pass1 and not pass3:
            @pl.when(t == 0)
            def _():
                cp_o.wait()
        KS1 = (NP // 2) * PW
        acc_ref[0:RW] = _dot_out(o_ref[0:RW, 0:KS1], wo_ref[0:KS1, :])
        pv(NP - 1, s0, s1, v)
        aout = acc_ref[0:RW] + _dot_out(o_ref[0:RW, KS1:], wo_ref[KS1:, :])

        if full:
            x1 = (r_ref[seg(t), :].astype(F32) + aout[T1:T3]).astype(BF16)
            x3 = (r_ref[seg(t - 2), :].astype(F32) + aout[T3:T4]).astype(BF16)
            r_ref[seg(t), :] = x1
            r_ref[seg(t - 2), :] = x3
        else:
            sg = seg(t - 2 * lay)
            r_ref[sg, :] = (r_ref[sg, :].astype(F32) + aout[T1:T3]).astype(BF16)
            x1 = r_ref[seg(t), :]
            x3 = r_ref[seg(t - 2), :]
        mrow = lax.broadcasted_iota(I32, (T1, D), 0)
        keep = (mrow < M) | (t >= 2)
        h_ref[nslot, 0:T1, :] = jnp.where(keep, aout[0:T1], mem00).astype(BF16)
        h_ref[nslot, T1:T3, :] = _ln(r_ref[seg(t + 1), :].astype(F32)).astype(BF16)

        x2 = b_out(t, ob)
        h_ref[nslot, T3:T4, :] = _ln(x2.astype(F32)).astype(BF16)
        b_qkv(x1, x3)
        if pass3:
            @pl.when(t >= 3)
            def _():
                out_copy(t - 3).start()

    def out_copy(i):
        return pltpu.make_async_copy(r_ref.at[seg(i)], out_hbm.at[pl.ds(pl.multiple_of(i * SEG, SEG), SEG)],
                                     sems.at[5])

    def loop(lo, hi, *cfg):
        def body(t, _):
            step(t, *cfg)
            return 0
        lax.fori_loop(lo, hi, body, 0)

    loop(0, 2, False, False, 0)
    loop(2, NPRE, False, True, None)
    loop(NPRE, NS, True, True, None)
    loop(NS, NS + 2, False, True, 1)
    b_out(NS + 2, b_local_attn(NS + 2))
    out_copy(NS - 1).start()
    pltpu.make_async_copy(r_ref.at[PAD * SEG:(PAD + NS) * SEG], out_hbm, sems.at[5]).wait()


@functools.partial(jax.jit, static_argnames=("A_seg_len",))
def pallas_interleave_layers__memory_aug_recurrent_mem_tr__sliding_local_dilated__prompt_kernel(A_x, A_mem0, A_Wq, A_Wk, A_Wv, A_Wo, A_seg_len, B_x, B_wqkv, B_wo):
    del B_x
    B, S, D = A_x.shape
    M = A_mem0.shape[1]
    _, H, DH = A_Wq.shape
    SEG = A_seg_len
    HD = H * DH
    x = A_x.reshape(S, D)
    mem0 = A_mem0.reshape(M, D)
    wq = jnp.transpose(A_Wq, (1, 2, 0)).reshape(HD, D)
    wk = jnp.transpose(A_Wk, (1, 2, 0)).reshape(HD, D)
    wv = jnp.transpose(A_Wv, (1, 2, 0)).reshape(HD, D)
    wo = A_Wo.reshape(HD, D)
    R2 = 2 * M + 2 * SEG
    NPRE = 6
    kern = functools.partial(_kernel, S=S, D=D, H=H, DH=DH, M=M, SEG=SEG, BH=32, BW=8, BDIL=2, NPRE=NPRE)
    out = pl.pallas_call(
        kern,
        out_shape=jax.ShapeDtypeStruct((S, D), BF16),
        in_specs=[pl.BlockSpec(memory_space=pl.ANY), pl.BlockSpec(memory_space=pltpu.VMEM)]
        + [pl.BlockSpec(memory_space=pl.ANY)] * 6,
        scratch_shapes=[
            pltpu.VMEM((S + 6 * SEG, D), BF16),
            pltpu.VMEM((2, R2, D), BF16),
            pltpu.VMEM((R2, HD), BF16),
            pltpu.VMEM((D, 3 * D), BF16),
            pltpu.VMEM((D, D), BF16),
            pltpu.VMEM((2, D // 128, SEG, 128), F32),
            pltpu.VMEM((2, D // 128, 16 + SEG, 128), F32),
            pltpu.VMEM((2, D // 128, 16 + SEG, 128), F32),
            pltpu.VMEM((R2, D), F32),
            pltpu.VMEM((HD, D), BF16),
            pltpu.VMEM((HD, D), BF16),
            pltpu.VMEM((HD, D), BF16),
            pltpu.VMEM((D, HD), BF16),
            pltpu.VMEM((D, HD), BF16),
            pltpu.VMEM((D, HD), BF16),
            pltpu.VMEM((HD, D), BF16),
            pltpu.VMEM((D, 3 * D), BF16),
            pltpu.VMEM((D, D), BF16),
            pltpu.VMEM((NPRE * SEG, D), BF16),
            pltpu.VMEM((NPRE * SEG, HD), BF16),
            pltpu.VMEM((NPRE * SEG, HD), BF16),
            pltpu.VMEM((NPRE * SEG, HD), BF16),
            pltpu.SemaphoreType.DMA((6,)),
            pltpu.SemaphoreType.DMA((H // 2,)),
        ],
        out_specs=pl.BlockSpec(memory_space=pl.ANY),
        compiler_params=pltpu.CompilerParams(vmem_limit_bytes=112 * 2**20),
    )(x, mem0, wq, wk, wv, wo, B_wqkv, B_wo)
    return out.reshape(B, S, D)
```

```python
import functools
import jax
import jax.numpy as jnp
from jax import lax
from jax.experimental import pallas as pl
from jax.experimental.pallas import tpu as pltpu

F32 = jnp.float32
BF16 = jnp.bfloat16
I32 = jnp.int32
NT_DIMS = (((1,), (1,)), ((), ()))
NEG = -1e9
EPS = 1e-5


def _ln(xf):
    m = jnp.mean(xf, axis=-1, keepdims=True)
    d = xf - m
    v = jnp.mean(d * d, axis=-1, keepdims=True)
    return d * lax.rsqrt(v + EPS)


def _dot(a, b):
    return jnp.dot(a, b, preferred_element_type=F32)


def _dot_nt(a, b):
    return lax.dot_general(a, b, NT_DIMS, preferred_element_type=F32)


def _dot_nn(a, b):
    return jnp.dot(a, b, preferred_element_type=F32)


def _dot_qk(a, b):
    return lax.dot_general(a, b, NT_DIMS, preferred_element_type=F32)


def _dot_pv(a, b):
    return jnp.dot(a, b, preferred_element_type=F32)


def _dot_out(a, b):
    return jnp.dot(a, b, preferred_element_type=F32)


def _dot_bo(a, b):
    return jnp.dot(a, b, preferred_element_type=F32)


def _dot_bqkv(a, b):
    return jnp.dot(a, b, preferred_element_type=F32)


def _kernel(x_hbm, mem0_ref, wq_hbm, wk_hbm, wv_hbm, wo_hbm, bw_hbm, bo_hbm, out_hbm,
            r_ref, h_ref, o_ref, bwp_ref, bop_ref, qb_ref, kb_ref, vb_ref, acc_ref,
            sq_ref, sk_ref, sv_ref, wq_ref, wk_ref, wv_ref, wo_ref, bw_ref, bo_ref,
            hpre_ref, pq_ref, pk_ref, pv_ref, sems, psems,
            *, S, D, H, DH, M, SEG, BH, BW, BDIL, NPRE):
    NS = S // SEG
    NP = H // 2
    PW = 2 * DH
    R2 = 2 * M + 2 * SEG
    PAD = 3
    BDH = D // BH
    HALO = 16
    NT = D // 128
    T1, T3, T4 = 2 * M, 2 * M + SEG, 2 * M + 2 * SEG
    NK = T4 + T1
    a_scale = DH ** -0.5
    b_scale = BDH ** -0.5
    AHEAD = 8
    XH = (NPRE + 1) * SEG

    cp_bw = pltpu.make_async_copy(bw_hbm, bw_ref, sems.at[0])
    cp_bo = pltpu.make_async_copy(bo_hbm, bo_ref, sems.at[1])
    cp_xh = pltpu.make_async_copy(x_hbm.at[0:XH], r_ref.at[PAD * SEG:PAD * SEG + XH], sems.at[2])
    cp_xt = pltpu.make_async_copy(x_hbm.at[XH:S], r_ref.at[PAD * SEG + XH:PAD * SEG + S], sems.at[3])
    cp_o = pltpu.make_async_copy(wo_hbm, wo_ref, sems.at[4])

    def pair_copies(p):
        rows = pl.ds(pl.multiple_of(p * PW, PW), PW)
        return [pltpu.make_async_copy(w.at[rows], s.at[rows], psems.at[p])
                for w, s in ((wq_hbm, sq_ref), (wk_hbm, sk_ref), (wv_hbm, sv_ref))]

    cp_bw.start()
    cp_bo.start()
    cp_xh.start()
    cp_bw.wait()
    cp_bo.wait()
    for p in range(AHEAD):
        for cp in pair_copies(p):
            cp.start()

    rr = lax.broadcasted_iota(I32, (D, D), 0)
    cc = lax.broadcasted_iota(I32, (D, D), 1)
    src_of_c = (cc % BH) * BDH + cc // BH
    perm = jnp.where(rr == src_of_c, 1.0, 0.0).astype(BF16)
    src_of_r = (rr % BH) * BDH + rr // BH
    permT = jnp.where(cc == src_of_r, 1.0, 0.0).astype(BF16)
    for i in range(3):
        bwp_ref[:, i * D:(i + 1) * D] = _dot(bw_ref[:, i * D:(i + 1) * D], perm).astype(BF16)
    bop_ref[...] = _dot(permT, bo_ref[...]).astype(BF16)

    r_ref[0:PAD * SEG, :] = jnp.zeros((PAD * SEG, D), BF16)
    r_ref[(PAD + NS) * SEG:(2 * PAD + NS) * SEG, :] = jnp.zeros((PAD * SEG, D), BF16)
    qb_ref[...] = jnp.zeros(qb_ref.shape, F32)
    kb_ref[...] = jnp.zeros(kb_ref.shape, F32)
    vb_ref[...] = jnp.zeros(vb_ref.shape, F32)

    mem0 = mem0_ref[...].astype(F32)
    mem00 = jnp.concatenate([mem0, mem0], axis=0)
    h_ref[0, 0:T1, :] = mem00.astype(BF16)
    cp_xh.wait()
    hpre_ref[...] = _ln(r_ref[PAD * SEG:(PAD + NPRE) * SEG, :].astype(F32)).astype(BF16)

    def pair_prologue(p, _):
        for cp in pair_copies(p):
            cp.wait()

        @pl.when(p + AHEAD < NP)
        def _():
            for cp in pair_copies(p + AHEAD):
                cp.start()

        @pl.when(p + AHEAD == NP)
        def _():
            cp_o.start()
            cp_xt.start()

        rows = pl.ds(pl.multiple_of(p * PW, PW), PW)
        cols = pl.ds(pl.multiple_of(p * PW, 128), PW)
        hp = hpre_ref[...]
        for s_ref, w_ref, p_ref in ((sq_ref, wq_ref, pq_ref), (sk_ref, wk_ref, pk_ref),
                                    (sv_ref, wv_ref, pv_ref)):
            w = s_ref[rows, :]
            p_ref[:, cols] = _dot_nt(hp, w).astype(BF16)
            w_ref[:, cols] = w.T
        return 0

    lax.fori_loop(0, NP, pair_prologue, 0)

    def seg(i):
        return pl.ds(pl.multiple_of((i + PAD) * SEG, SEG), SEG)

    def b_local_attn(t):
        blocks = []
        for l, sidx in enumerate((t - 1, t - 3)):
            for rb in range(SEG // 8):
                pos = lax.broadcasted_iota(I32, (8, 128), 0) + (sidx * SEG + rb * 8)
                qs = [qb_ref[l, c, rb * 8:rb * 8 + 8, :] for c in range(NT)]
                logits = []
                for w in range(BW):
                    r0 = HALO - BDIL * w + rb * 8
                    a = None
                    for c in range(NT):
                        pr = qs[c] * kb_ref[l, c, r0:r0 + 8, :]
                        a = pr if a is None else a + pr
                    a = a + pltpu.roll(a, 64, 1)
                    a = a + pltpu.roll(a, 32, 1)
                    logits.append(jnp.where(pos >= BDIL * w, a, NEG))
                mx = logits[0]
                for w in range(1, BW):
                    mx = jnp.maximum(mx, logits[w])
                es = [jnp.exp(a - mx) for a in logits]
                sm = es[0]
                for w in range(1, BW):
                    sm = sm + es[w]
                inv = 1.0 / sm
                aws = [e * inv for e in es]
                tiles = []
                for c in range(NT):
                    ob = None
                    for w in range(BW):
                        r0 = HALO - BDIL * w + rb * 8
                        term = aws[w] * vb_ref[l, c, r0:r0 + 8, :]
                        ob = term if ob is None else ob + term
                    tiles.append(ob)
                blocks.append(jnp.concatenate(tiles, axis=1))
        return jnp.concatenate(blocks, axis=0).astype(BF16)

    def b_out(t, ob):
        bout = _dot_bo(ob, bop_ref[...])
        x2 = (r_ref[seg(t - 1), :].astype(F32) + bout[0:SEG]).astype(BF16)
        r_ref[seg(t - 1), :] = x2
        r_ref[seg(t - 3), :] = (r_ref[seg(t - 3), :].astype(F32) + bout[SEG:2 * SEG]).astype(BF16)
        return x2

    def b_qkv(xa, xb):
        hb = jnp.concatenate([_ln(xa.astype(F32)), _ln(xb.astype(F32))], axis=0).astype(BF16)
        qkv = _dot_bqkv(hb, bwp_ref[...])
        for l in range(2):
            rows = slice(l * SEG, (l + 1) * SEG)
            for c in range(NT):
                cs = slice(c * 128, (c + 1) * 128)
                qb_ref[l, c] = qkv[rows, cs] * b_scale
                kb_ref[l, c, 0:HALO, :] = kb_ref[l, c, SEG:SEG + HALO, :]
                vb_ref[l, c, 0:HALO, :] = vb_ref[l, c, SEG:SEG + HALO, :]
                kb_ref[l, c, HALO:HALO + SEG, :] = qkv[rows, D + c * 128:D + (c + 1) * 128]
                vb_ref[l, c, HALO:HALO + SEG, :] = qkv[rows, 2 * D + c * 128:2 * D + (c + 1) * 128]

    def softmax(s, mask):
        s = jnp.where(mask, s * a_scale, NEG)
        mx = jnp.max(s, axis=-1, keepdims=True)
        e = jnp.exp(s - mx)
        sm = jnp.sum(e, axis=-1, keepdims=True)
        return e * (1.0 / sm)

    def split_lo_hi(z):
        rows = z.shape[0]
        lo32 = jnp.where(lax.broadcasted_iota(I32, (rows // 2, 128), 1) < 64, I32(-1), I32(0))
        zi = pltpu.bitcast(z, I32)
        return pltpu.bitcast(zi & lo32, BF16), pltpu.bitcast(zi & ~lo32, BF16)

    def step(t, pass1, pass3, active, LAG=1):
        slot = lax.rem(t, 2)
        nslot = 1 - slot
        full = active is None
        lay = active
        RW = R2 if full else T3
        parts = [h_ref[slot, 0:T1, :]]
        if pass1:
            parts.append(h_ref[slot, T1:T3, :])
        if pass3:
            parts.append(h_ref[slot, T3:T4, :])
        hrows = h_ref[slot] if (pass1 and pass3) else jnp.concatenate(parts, axis=0)

        ri = lax.broadcasted_iota(I32, (RW, NK), 0)
        ci = lax.broadcasted_iota(I32, (RW, NK), 1)
        if full:
            def layer(i):
                return jnp.where(i < M, 0, jnp.where(i < T1, 1, jnp.where(i < T3, 0, 1)))
            def allowed(kidx, kvalid):
                return kvalid & (layer(ri) == layer(kidx)) & ((ri < T1) | (kidx < T1) | (ri >= kidx))
            mask0 = allowed(ci, ci < T4)
            nat1 = jnp.where(ci < T3, ci - T1 + T3, jnp.where(ci < T4, ci - T3 + T1, ci - T4))
            mask1 = allowed(nat1, ci >= T1)
        else:
            def allowed(kidx, kvalid):
                kok = kvalid & ((kidx >= T1) | (kidx // M == lay))
                return kok & ((ri < T1) | (kidx < T1) | (ri >= kidx))
            mask0 = allowed(ci, ci < T3)
            nat1 = jnp.where(ci < T4, ci - T3 + T1, ci - T4)
            mask1 = allowed(nat1, ci >= T3)

        def proj(w_ref, pre_ref, p):
            c0 = p * PW
            y = _dot_nn(hrows, w_ref[:, c0:c0 + PW]).astype(BF16)
            if pass1 or lay == 1:
                return y
            pre = pre_ref[pl.ds(pl.multiple_of(t * SEG, SEG), SEG), c0:c0 + PW]
            if pass3:
                return jnp.concatenate([y[0:T1], pre, y[T1:T3]], axis=0)
            return jnp.concatenate([y, pre], axis=0)

        if full:
            def b_weights(z):
                zl, zh = split_lo_hi(z)
                w1 = jnp.concatenate([zl[0:T3], zh[T1:T3], zh[0:T1]], axis=0)
                w3 = jnp.concatenate([zl[0:T1], zh[T3:T4], zl[T3:T4], zh[0:T1]], axis=0)
                return w1, w3

            def h0_rows(z):
                return jnp.concatenate([z, z[0:T1]], axis=0)

            def h1_rows(z):
                return jnp.concatenate([z[0:T1], z[T3:T4], z[T1:T3], z[0:T1]], axis=0)

            def shared(dot, lhs, ws):
                y1 = dot(lhs[0:T3], ws[0])
                y3 = dot(jnp.concatenate([lhs[0:T1], lhs[T3:T4]], axis=0), ws[1])
                return jnp.concatenate([y1[0:M], y3[M:T1], y1[T1:T3], y3[T1:T3]], axis=0)
        else:
            def b_weights(z):
                zl, zh = split_lo_hi(z)
                return (jnp.concatenate([zl, zh[T1:T3], zh[0:T1]], axis=0),)

            def h0_rows(z):
                return jnp.concatenate([z, z], axis=0)

            def h1_rows(z):
                return jnp.concatenate([z, z[T1:T3], z[0:T1]], axis=0)

            def shared(dot, lhs, ws):
                return dot(lhs, ws[0])

        def qk(q, k):
            qA, qB, qC = q[:, 0:128], q[:, 128:256], q[:, 256:384]
            sa = _dot_qk(qA, h0_rows(k[:, 0:128]))
            sc = _dot_qk(qC, h1_rows(k[:, 256:384]))
            x = shared(_dot_qk, qB, b_weights(k[:, 128:256]))
            return sa + x, sc + x

        def pv(p, s0, s1, v):
            c0 = p * PW
            p0 = softmax(s0, mask0)
            p1 = softmax(s1, mask1)
            pm = (p0 + p1).astype(BF16)
            oa = _dot_pv(p0.astype(BF16), h0_rows(v[:, 0:128]))
            oc = _dot_pv(p1.astype(BF16), h1_rows(v[:, 256:384]))
            ob_ = shared(_dot_pv, pm, b_weights(v[:, 128:256]))
            o_ref[0:RW, c0:c0 + 128] = oa.astype(BF16)
            o_ref[0:RW, c0 + 128:c0 + 256] = ob_.astype(BF16)
            o_ref[0:RW, c0 + 256:c0 + 384] = oc.astype(BF16)

        if not pass1 and not pass3:
            @pl.when(t == 1)
            def _():
                cp_xt.wait()

        ob = b_local_attn(t)

        qs, ks, vs, ss = {}, {}, {}, {}
        first = NP // 2 if LAG == 1 else (NP - LAG) // 2
        cuts = [0, first] + [first + ((NP - LAG + s) - first) * 1 for s in range(1, LAG)]
        def out_chunk(c0, c1):
            return _dot_out(o_ref[0:RW, c0 * PW:c1 * PW], wo_ref[c0 * PW:c1 * PW, :])
        for p in range(NP + LAG):
            if 1 <= p <= NP:
                ss[p - 1] = qk(qs.pop(p - 1), ks.pop(p - 1))
            if p < NP:
                qs[p] = proj(wq_ref, pq_ref, p)
                ks[p] = proj(wk_ref, pk_ref, p)
            else:
                s = p - NP
                if s == 0:
                    if not pass1 and not pass3:
                        @pl.when(t == 0)
                        def _():
                            cp_o.wait()
                    acc_ref[0:RW] = out_chunk(cuts[0], cuts[1])
                else:
                    acc_ref[0:RW] += out_chunk(cuts[s], cuts[s + 1])
            if p >= LAG:
                pv(p - LAG, *ss.pop(p - LAG), vs.pop(p - LAG))
            if p < NP:
                vs[p] = proj(wv_ref, pv_ref, p)
        aout = acc_ref[0:RW] + out_chunk(cuts[LAG], NP)

        if full:
            x1 = (r_ref[seg(t), :].astype(F32) + aout[T1:T3]).astype(BF16)
            x3 = (r_ref[seg(t - 2), :].astype(F32) + aout[T3:T4]).astype(BF16)
            r_ref[seg(t), :] = x1
            r_ref[seg(t - 2), :] = x3
        else:
            sg = seg(t - 2 * lay)
            r_ref[sg, :] = (r_ref[sg, :].astype(F32) + aout[T1:T3]).astype(BF16)
            x1 = r_ref[seg(t), :]
            x3 = r_ref[seg(t - 2), :]
        mrow = lax.broadcasted_iota(I32, (T1, D), 0)
        keep = (mrow < M) | (t >= 2)
        h_ref[nslot, 0:T1, :] = jnp.where(keep, aout[0:T1], mem00).astype(BF16)
        h_ref[nslot, T1:T3, :] = _ln(r_ref[seg(t + 1), :].astype(F32)).astype(BF16)

        x2 = b_out(t, ob)
        h_ref[nslot, T3:T4, :] = _ln(x2.astype(F32)).astype(BF16)
        b_qkv(x1, x3)
        if pass3:
            @pl.when(t >= 3)
            def _():
                out_copy(t - 3).start()

    def out_copy(i):
        return pltpu.make_async_copy(r_ref.at[seg(i)], out_hbm.at[pl.ds(pl.multiple_of(i * SEG, SEG), SEG)],
                                     sems.at[5])

    def loop(lo, hi, *cfg, unroll=1):
        def body(i, _):
            for u in range(unroll):
                step(lo + i * unroll + u, *cfg)
            return 0
        assert (hi - lo) % unroll == 0
        lax.fori_loop(0, (hi - lo) // unroll, body, 0)

    loop(0, 2, False, False, 0, 4)
    loop(2, NPRE, False, True, None, 3)
    loop(NPRE, NS, True, True, None, unroll=2)
    loop(NS, NS + 2, False, True, 1, 3)
    b_out(NS + 2, b_local_attn(NS + 2))
    out_copy(NS - 1).start()
    pltpu.make_async_copy(r_ref.at[PAD * SEG:(PAD + NS) * SEG], out_hbm, sems.at[5]).wait()


@functools.partial(jax.jit, static_argnames=("A_seg_len",))
def pallas_interleave_layers__memory_aug_recurrent_mem_tr__sliding_local_dilated__prompt_kernel(A_x, A_mem0, A_Wq, A_Wk, A_Wv, A_Wo, A_seg_len, B_x, B_wqkv, B_wo):
    del B_x
    B, S, D = A_x.shape
    M = A_mem0.shape[1]
    _, H, DH = A_Wq.shape
    SEG = A_seg_len
    HD = H * DH
    x = A_x.reshape(S, D)
    mem0 = A_mem0.reshape(M, D)
    wq = jnp.transpose(A_Wq, (1, 2, 0)).reshape(HD, D)
    wk = jnp.transpose(A_Wk, (1, 2, 0)).reshape(HD, D)
    wv = jnp.transpose(A_Wv, (1, 2, 0)).reshape(HD, D)
    wo = A_Wo.reshape(HD, D)
    R2 = 2 * M + 2 * SEG
    NPRE = 6
    kern = functools.partial(_kernel, S=S, D=D, H=H, DH=DH, M=M, SEG=SEG, BH=32, BW=8, BDIL=2, NPRE=NPRE)
    out = pl.pallas_call(
        kern,
        out_shape=jax.ShapeDtypeStruct((S, D), BF16),
        in_specs=[pl.BlockSpec(memory_space=pl.ANY), pl.BlockSpec(memory_space=pltpu.VMEM)]
        + [pl.BlockSpec(memory_space=pl.ANY)] * 6,
        scratch_shapes=[
            pltpu.VMEM((S + 6 * SEG, D), BF16),
            pltpu.VMEM((2, R2, D), BF16),
            pltpu.VMEM((R2, HD), BF16),
            pltpu.VMEM((D, 3 * D), BF16),
            pltpu.VMEM((D, D), BF16),
            pltpu.VMEM((2, D // 128, SEG, 128), F32),
            pltpu.VMEM((2, D // 128, 16 + SEG, 128), F32),
            pltpu.VMEM((2, D // 128, 16 + SEG, 128), F32),
            pltpu.VMEM((R2, D), F32),
            pltpu.VMEM((HD, D), BF16),
            pltpu.VMEM((HD, D), BF16),
            pltpu.VMEM((HD, D), BF16),
            pltpu.VMEM((D, HD), BF16),
            pltpu.VMEM((D, HD), BF16),
            pltpu.VMEM((D, HD), BF16),
            pltpu.VMEM((HD, D), BF16),
            pltpu.VMEM((D, 3 * D), BF16),
            pltpu.VMEM((D, D), BF16),
            pltpu.VMEM((NPRE * SEG, D), BF16),
            pltpu.VMEM((NPRE * SEG, HD), BF16),
            pltpu.VMEM((NPRE * SEG, HD), BF16),
            pltpu.VMEM((NPRE * SEG, HD), BF16),
            pltpu.SemaphoreType.DMA((6,)),
            pltpu.SemaphoreType.DMA((H // 2,)),
        ],
        out_specs=pl.BlockSpec(memory_space=pl.ANY),
        compiler_params=pltpu.CompilerParams(vmem_limit_bytes=112 * 2**20),
    )(x, mem0, wq, wk, wv, wo, B_wqkv, B_wo)
    return out.reshape(B, S, D)
```

```python
import functools

import jax
import jax.numpy as jnp
from jax import lax
from jax.experimental import pallas as pl
from jax.experimental.pallas import tpu as pltpu

F32 = jnp.float32
BF16 = jnp.bfloat16
I32 = jnp.int32
NT_DIMS = (((1,), (1,)), ((), ()))
NEG = -1e9
EPS = 1e-5


LOCAL_HEADS, LOCAL_WINDOW, LOCAL_DILATION = 32, 8, 2
NPRE = 10
AHEAD = 3
BW_AT = 12
WO_AT = 13
LAG_A, LAG_B, LAG_F, LAG_E = 4, 3, 1, 3
UNROLL = 1


def _ln(xf):
    m = jnp.mean(xf, axis=-1, keepdims=True)
    d = xf - m
    v = jnp.mean(d * d, axis=-1, keepdims=True)
    return d * lax.rsqrt(v + EPS)


def _dot(a, b):
    return jnp.dot(a, b, preferred_element_type=F32)


def _dot_nt(a, b):
    return lax.dot_general(a, b, NT_DIMS, preferred_element_type=F32)


def _unpack(w32):
    return pltpu.bitcast(w32, BF16)


def _kernel(x_hbm, mem0_ref, wq_hbm, wk_hbm, wv_hbm, wo_hbm, bw_hbm, bo_hbm, out_hbm,
            r_ref, h_ref, o_ref, bwp_ref, bop_ref, qb_ref, kb_ref, vb_ref, acc_ref,
            sq_ref, sk_ref, sv_ref, wq_ref, wk_ref, wv_ref, wo_ref, bw_ref, bo_ref,
            hpre_ref, pq_ref, pk_ref, pv_ref, tr_ref, sems, psems,
            *, S, D, H, DH, M, SEG):
    BH, BW, BDIL = LOCAL_HEADS, LOCAL_WINDOW, LOCAL_DILATION
    NS = S // SEG
    NP = H // 2
    PW = 2 * DH
    T1, T3, T4 = 2 * M, 2 * M + SEG, 2 * M + 2 * SEG
    NK = T4 + T1
    PAD = 3
    BDH = D // BH
    HALO = 16
    NT = D // 128
    a_scale = DH ** -0.5
    b_scale = BDH ** -0.5
    XH = (NPRE + 1) * SEG

    cp_bw = pltpu.make_async_copy(bw_hbm, bw_ref, sems.at[0])
    cp_bo = pltpu.make_async_copy(bo_hbm, bo_ref, sems.at[1])
    cp_xh = pltpu.make_async_copy(x_hbm.at[0:XH], r_ref.at[PAD * SEG:PAD * SEG + XH], sems.at[2])
    cp_xt = pltpu.make_async_copy(x_hbm.at[XH:S], r_ref.at[PAD * SEG + XH:PAD * SEG + S], sems.at[3])
    cp_wo = pltpu.make_async_copy(wo_hbm, wo_ref, sems.at[4])

    def pair_copies(p):
        rows = pl.ds(pl.multiple_of(p * PW, PW), PW)
        return [pltpu.make_async_copy(w.at[rows], s.at[rows], psems.at[p])
                for w, s in ((wq_hbm, sq_ref), (wk_hbm, sk_ref), (wv_hbm, sv_ref))]

    def seg(i):
        return pl.ds(pl.multiple_of((i + PAD) * SEG, SEG), SEG)

    def out_copy(i):
        return pltpu.make_async_copy(
            r_ref.at[seg(i)], out_hbm.at[pl.ds(pl.multiple_of(i * SEG, SEG), SEG)], sems.at[5])

    cp_xh.start()
    for p in range(AHEAD):
        for cp in pair_copies(p):
            cp.start()

    r_ref[0:PAD * SEG, :] = jnp.zeros((PAD * SEG, D), BF16)
    r_ref[(PAD + NS) * SEG:(2 * PAD + NS) * SEG, :] = jnp.zeros((PAD * SEG, D), BF16)
    qb_ref[...] = jnp.zeros(qb_ref.shape, F32)
    kb_ref[...] = jnp.zeros(kb_ref.shape, F32)
    vb_ref[...] = jnp.zeros(vb_ref.shape, F32)
    mem0 = mem0_ref[...].astype(F32)
    mem00 = jnp.concatenate([mem0, mem0], axis=0)
    h_ref[0, 0:T1, :] = mem00.astype(BF16)
    cp_xh.wait()
    hpre_ref[...] = _ln(r_ref[PAD * SEG:(PAD + NPRE) * SEG, :].astype(F32)).astype(BF16)

    def pair_prologue(p, _):
        for cp in pair_copies(p):
            cp.wait()

        @pl.when(p + AHEAD < NP)
        def _():
            for cp in pair_copies(p + AHEAD):
                cp.start()

        @pl.when(p == BW_AT)
        def _():
            cp_bw.start()
            cp_bo.start()

        @pl.when(p == WO_AT)
        def _():
            cp_wo.start()

        rows = pl.ds(pl.multiple_of(p * PW, PW), PW)
        cols = pl.ds(pl.multiple_of(p * PW, 128), PW)
        hp = hpre_ref[0:(NPRE - 2) * SEG, :]
        for s_ref, w_ref, p_ref in ((sq_ref, wq_ref, pq_ref), (sk_ref, wk_ref, pk_ref),
                                    (sv_ref, wv_ref, pv_ref)):
            w = s_ref[rows, :]
            p_ref[0:(NPRE - 2) * SEG, cols] = _dot_nt(hp, w).astype(BF16)
            w_ref[:, cols] = pltpu.bitcast(w.T, I32)
        return 0

    lax.fori_loop(0, NP, pair_prologue, 0)

    def gather_rows(base):
        return jnp.concatenate(
            [tr_ref[pl.ds(base + j, BH, stride=BDH), :] for j in range(BDH)], axis=0)

    cp_bw.wait()
    cp_bo.wait()
    tr_ref[3 * D:3 * D + BH, :] = jnp.zeros((BH, 128), F32)
    for kt in range(NT):
        tr_ref[0:3 * D, :] = bw_ref[kt * 128:(kt + 1) * 128, :].T.astype(F32)
        for i in range(3):
            g = gather_rows(i * D).astype(BF16).T
            bwp_ref[kt * 64:(kt + 1) * 64, i * D:(i + 1) * D] = pltpu.bitcast(g, I32)
    for lt in range(NT):
        tr_ref[0:D, :] = bo_ref[:, lt * 128:(lt + 1) * 128].astype(F32)
        bop_ref[:, lt * 128:(lt + 1) * 128] = pltpu.bitcast(gather_rows(0).astype(BF16), I32)

    def b_seg(t, l):
        return t - 1 - 2 * l

    def b_local_attn(t, slots):
        blocks = []
        for l in slots:
            for rb in range(SEG // 8):
                pos = lax.broadcasted_iota(I32, (8, 128), 0) + (b_seg(t, l) * SEG + rb * 8)
                qs = [qb_ref[l, c, rb * 8:rb * 8 + 8, :] for c in range(NT)]
                logits = []
                for w in range(BW):
                    r0 = HALO - BDIL * w + rb * 8
                    a = None
                    for c in range(NT):
                        pr = qs[c] * kb_ref[l, c, r0:r0 + 8, :]
                        a = pr if a is None else a + pr
                    a = a + pltpu.roll(a, 64, 1)
                    a = a + pltpu.roll(a, 32, 1)
                    logits.append(jnp.where(pos >= BDIL * w, a, NEG))
                mx = logits[0]
                for w in range(1, BW):
                    mx = jnp.maximum(mx, logits[w])
                es = [jnp.exp(a - mx) for a in logits]
                sm = es[0]
                for w in range(1, BW):
                    sm = sm + es[w]
                inv = 1.0 / sm
                aws = [e * inv for e in es]
                tiles = []
                for c in range(NT):
                    ob = None
                    for w in range(BW):
                        r0 = HALO - BDIL * w + rb * 8
                        term = aws[w] * vb_ref[l, c, r0:r0 + 8, :]
                        ob = term if ob is None else ob + term
                    tiles.append(ob)
                blocks.append(jnp.concatenate(tiles, axis=1))
        return jnp.concatenate(blocks, axis=0).astype(BF16)

    def b_out(t, slots, ob):
        bout = _dot(ob, _unpack(bop_ref[...]))
        news = []
        for i, l in enumerate(slots):
            sg = seg(b_seg(t, l))
            new = (r_ref[sg, :].astype(F32) + bout[i * SEG:(i + 1) * SEG]).astype(BF16)
            r_ref[sg, :] = new
            news.append(new)
        return news

    def b_qkv(slots, xs):
        hb = jnp.concatenate([_ln(x.astype(F32)) for x in xs], axis=0).astype(BF16)
        qkv = _dot(hb, _unpack(bwp_ref[...]))
        for i, l in enumerate(slots):
            rows = slice(i * SEG, (i + 1) * SEG)
            for c in range(NT):
                c0 = c * 128
                qb_ref[l, c] = qkv[rows, c0:c0 + 128] * b_scale
                kb_ref[l, c, 0:HALO, :] = kb_ref[l, c, SEG:SEG + HALO, :]
                vb_ref[l, c, 0:HALO, :] = vb_ref[l, c, SEG:SEG + HALO, :]
                kb_ref[l, c, HALO:HALO + SEG, :] = qkv[rows, D + c0:D + c0 + 128]
                vb_ref[l, c, HALO:HALO + SEG, :] = qkv[rows, 2 * D + c0:2 * D + c0 + 128]

    def softmax(s, mask):
        s = jnp.where(mask, s * a_scale, NEG)
        mx = jnp.max(s, axis=-1, keepdims=True)
        e = jnp.exp(s - mx)
        sm = jnp.sum(e, axis=-1, keepdims=True)
        return e * (1.0 / sm)

    def split_lo_hi(z):
        rows = z.shape[0]
        lo32 = jnp.where(lax.broadcasted_iota(I32, (rows // 2, 128), 1) < 64, I32(-1), I32(0))
        zi = pltpu.bitcast(z, I32)
        return pltpu.bitcast(zi & lo32, BF16), pltpu.bitcast(zi & ~lo32, BF16)

    def step(t, kind, lag):
        slot = lax.rem(t, 2)
        nslot = 1 - slot
        both = kind in ("ramp", "full")
        lay = 0 if kind == "head" else 1
        RW = T4 if both else T3
        if kind == "full":
            hrows = h_ref[slot]
        elif kind == "head":
            arows = pl.ds(pl.multiple_of((NPRE - 2 + t) * SEG, SEG), SEG)
            hrows = jnp.concatenate([h_ref[slot, 0:T1, :], hpre_ref[arows, :]], axis=0)
        else:
            hrows = jnp.concatenate([h_ref[slot, 0:T1, :], h_ref[slot, T3:T4, :]], axis=0)
        b_attn_slots = {"head": (0,), "ramp": (0, 1), "full": (0, 1), "tail": (0, 1)}[kind]
        b_qkv_slots = {"head": (0,), "ramp": (0, 1), "full": (0, 1), "tail": (1,)}[kind]

        ri = lax.broadcasted_iota(I32, (RW, NK), 0)
        ci = lax.broadcasted_iota(I32, (RW, NK), 1)
        if both:
            def layer(i):
                return jnp.where(i < M, 0, jnp.where(i < T1, 1, jnp.where(i < T3, 0, 1)))

            def allowed(kidx, kvalid):
                return kvalid & (layer(ri) == layer(kidx)) & ((ri < T1) | (kidx < T1) | (ri >= kidx))
            mask0 = allowed(ci, ci < T4)
            nat1 = jnp.where(ci < T3, ci - T1 + T3, jnp.where(ci < T4, ci - T3 + T1, ci - T4))
            mask1 = allowed(nat1, ci >= T1)

            def shared_w(z):
                zl, zh = split_lo_hi(z)
                w1 = jnp.concatenate([zl[0:T3], zh[T1:T3], zh[0:T1]], axis=0)
                w3 = jnp.concatenate([zl[0:T1], zh[T3:T4], zl[T3:T4], zh[0:T1]], axis=0)
                return w1, w3

            def h0_rows(z):
                return jnp.concatenate([z, z[0:T1]], axis=0)

            def h1_rows(z):
                return jnp.concatenate([z[0:T1], z[T3:T4], z[T1:T3], z[0:T1]], axis=0)

            def shared(dot, lhs, ws):
                y1 = dot(lhs[0:T3], ws[0])
                y3 = dot(jnp.concatenate([lhs[0:T1], lhs[T3:T4]], axis=0), ws[1])
                return jnp.concatenate([y1[0:M], y3[M:T1], y1[T1:T3], y3[T1:T3]], axis=0)
        else:
            def allowed(kidx, kvalid):
                kok = kvalid & ((kidx >= T1) | (kidx // M == lay))
                return kok & ((ri < T1) | (kidx < T1) | (ri >= kidx))
            mask0 = allowed(ci, ci < T3)
            nat1 = jnp.where(ci < T4, ci - T3 + T1, ci - T4)
            mask1 = allowed(nat1, ci >= T3)

            def shared_w(z):
                zl, zh = split_lo_hi(z)
                return (jnp.concatenate([zl, zh[T1:T3], zh[0:T1]], axis=0),)

            def h0_rows(z):
                return jnp.concatenate([z, z], axis=0)

            def h1_rows(z):
                return jnp.concatenate([z, z[T1:T3], z[0:T1]], axis=0)

            def shared(dot, lhs, ws):
                return dot(lhs, ws[0])

        def proj(w_ref, pre_ref, p):
            c0 = p * PW
            y = _dot(hrows, _unpack(w_ref[:, c0:c0 + PW])).astype(BF16)
            if kind in ("full", "tail"):
                return y
            pre = pre_ref[pl.ds(pl.multiple_of(t * SEG, SEG), SEG), c0:c0 + PW]
            if kind == "ramp":
                return jnp.concatenate([y[0:T1], pre, y[T1:T3]], axis=0)
            pre_ref[arows, c0:c0 + PW] = y[T1:T3]
            return jnp.concatenate([y[0:T1], pre], axis=0)

        def qk(q, k):
            qA, qB, qC = q[:, 0:128], q[:, 128:256], q[:, 256:384]
            sa = _dot_nt(qA, h0_rows(k[:, 0:128]))
            sc = _dot_nt(qC, h1_rows(k[:, 256:384]))
            x = shared(_dot_nt, qB, shared_w(k[:, 128:256]))
            return sa + x, sc + x

        def pv(p, s0, s1, v):
            c0 = p * PW
            p0 = softmax(s0, mask0)
            p1 = softmax(s1, mask1)
            pm = (p0 + p1).astype(BF16)
            oa = _dot(p0.astype(BF16), h0_rows(v[:, 0:128]))
            oc = _dot(p1.astype(BF16), h1_rows(v[:, 256:384]))
            ob_ = shared(_dot, pm, shared_w(v[:, 128:256]))
            o_ref[0:RW, c0:c0 + 128] = oa.astype(BF16)
            o_ref[0:RW, c0 + 128:c0 + 256] = ob_.astype(BF16)
            o_ref[0:RW, c0 + 256:c0 + 384] = oc.astype(BF16)

        def out_chunk(c0, c1):
            return _dot(o_ref[0:RW, c0 * PW:c1 * PW], wo_ref[c0 * PW:c1 * PW, :])

        ob = b_local_attn(t, b_attn_slots)

        qs, ks, vs, ss = {}, {}, {}, {}
        cuts = [0, (NP + 1 - lag) // 2] + [NP - lag + s for s in range(1, lag)]
        for p in range(NP + lag):
            if 1 <= p <= NP:
                ss[p - 1] = qk(qs.pop(p - 1), ks.pop(p - 1))
            if p < NP:
                qs[p] = proj(wq_ref, pq_ref, p)
                ks[p] = proj(wk_ref, pk_ref, p)
            elif p == NP:
                if kind == "head":
                    @pl.when(t == 0)
                    def _():
                        cp_wo.wait()
                        cp_xt.start()
                acc_ref[0:RW] = out_chunk(cuts[0], cuts[1])
            else:
                acc_ref[0:RW] += out_chunk(cuts[p - NP], cuts[p - NP + 1])
            if p >= lag:
                pv(p - lag, *ss.pop(p - lag), vs.pop(p - lag))
            if p < NP:
                vs[p] = proj(wv_ref, pv_ref, p)
        aout = acc_ref[0:RW] + out_chunk(cuts[lag], NP)

        def add_residual(i, rows):
            new = (r_ref[seg(i), :].astype(F32) + aout[rows]).astype(BF16)
            r_ref[seg(i), :] = new
            return new

        if kind == "head":
            xs = [add_residual(t, slice(T1, T3))]
        elif kind == "tail":
            xs = [add_residual(t - 2, slice(T1, T3))]
        else:
            xs = [add_residual(t, slice(T1, T3)), add_residual(t - 2, slice(T3, T4))]
        mrow = lax.broadcasted_iota(I32, (T1, D), 0)
        keep = (mrow < M) | (t >= 2)
        h_ref[nslot, 0:T1, :] = jnp.where(keep, aout[0:T1], mem00).astype(BF16)
        if kind != "tail":
            h_ref[nslot, T1:T3, :] = _ln(r_ref[seg(t + 1), :].astype(F32)).astype(BF16)

        news = b_out(t, b_attn_slots, ob)
        h_ref[nslot, T3:T4, :] = _ln(news[0].astype(F32)).astype(BF16)
        b_qkv(b_qkv_slots, xs)
        if kind != "head":
            @pl.when(t >= 3)
            def _():
                out_copy(t - 3).start()

    def loop(lo, hi, kind, lag, unroll=1):
        assert (hi - lo) % unroll == 0

        def body(i, _):
            for u in range(unroll):
                step(lo + i * unroll + u, kind, lag)
            return 0
        lax.fori_loop(0, (hi - lo) // unroll, body, 0)

    loop(0, 2, "head", LAG_A)
    loop(2, NPRE, "ramp", LAG_B)
    cp_xt.wait()
    loop(NPRE, NS, "full", LAG_F, UNROLL)
    loop(NS, NS + 2, "tail", LAG_E)
    b_out(NS + 2, (1,), b_local_attn(NS + 2, (1,)))
    out_copy(NS - 1).start()
    pltpu.make_async_copy(r_ref.at[PAD * SEG:(PAD + NS) * SEG], out_hbm, sems.at[5]).wait()


@functools.partial(jax.jit, static_argnames=("A_seg_len",))
def pallas_interleave_layers__memory_aug_recurrent_mem_tr__sliding_local_dilated__prompt_kernel(A_x, A_mem0, A_Wq, A_Wk, A_Wv, A_Wo, A_seg_len, B_x, B_wqkv, B_wo):
    del B_x
    B, S, D = A_x.shape
    M = A_mem0.shape[1]
    _, H, DH = A_Wq.shape
    SEG = A_seg_len
    HD = H * DH
    x = A_x.reshape(S, D)
    mem0 = A_mem0.reshape(M, D)
    wq = jnp.transpose(A_Wq, (1, 2, 0)).reshape(HD, D)
    wk = jnp.transpose(A_Wk, (1, 2, 0)).reshape(HD, D)
    wv = jnp.transpose(A_Wv, (1, 2, 0)).reshape(HD, D)
    wo = A_Wo.reshape(HD, D)
    R2 = 2 * M + 2 * SEG
    kern = functools.partial(_kernel, S=S, D=D, H=H, DH=DH, M=M, SEG=SEG)
    hbm = pl.BlockSpec(memory_space=pl.ANY)
    out = pl.pallas_call(
        kern,
        out_shape=jax.ShapeDtypeStruct((S, D), BF16),
        in_specs=[hbm, pl.BlockSpec(memory_space=pltpu.VMEM)] + [hbm] * 6,
        out_specs=hbm,
        scratch_shapes=[
            pltpu.VMEM((S + 6 * SEG, D), BF16),
            pltpu.VMEM((2, R2, D), BF16),
            pltpu.VMEM((R2, HD), BF16),
            pltpu.VMEM((D // 2, 3 * D), I32),
            pltpu.VMEM((D // 2, D), I32),
            pltpu.VMEM((2, D // 128, SEG, 128), F32),
            pltpu.VMEM((2, D // 128, 16 + SEG, 128), F32),
            pltpu.VMEM((2, D // 128, 16 + SEG, 128), F32),
            pltpu.VMEM((R2, D), F32),
            pltpu.VMEM((HD, D), BF16),
            pltpu.VMEM((HD, D), BF16),
            pltpu.VMEM((HD, D), BF16),
            pltpu.VMEM((D // 2, HD), I32),
            pltpu.VMEM((D // 2, HD), I32),
            pltpu.VMEM((D // 2, HD), I32),
            pltpu.VMEM((HD, D), BF16),
            pltpu.VMEM((D, 3 * D), BF16),
            pltpu.VMEM((D, D), BF16),
            pltpu.VMEM((NPRE * SEG, D), BF16),
            pltpu.VMEM((NPRE * SEG, HD), BF16),
            pltpu.VMEM((NPRE * SEG, HD), BF16),
            pltpu.VMEM((NPRE * SEG, HD), BF16),
            pltpu.VMEM((3 * D + LOCAL_HEADS, 128), F32),
            pltpu.SemaphoreType.DMA((6,)),
            pltpu.SemaphoreType.DMA((H // 2,)),
        ],
        compiler_params=pltpu.CompilerParams(
            vmem_limit_bytes=120 * 2**20,
            flags={"XLA_TPU_EVENLY_DISTRIBUTE_CRITICAL_NODES": True}),
    )(x, mem0, wq, wk, wv, wo, B_wqkv, B_wo)
    return out.reshape(B, S, D)
```

```python
import functools

import jax
import jax.numpy as jnp
from jax import lax
from jax.experimental import pallas as pl
from jax.experimental.pallas import tpu as pltpu

F32 = jnp.float32
BF16 = jnp.bfloat16
I32 = jnp.int32
NT_DIMS = (((1,), (1,)), ((), ()))
NEG = -1e9
EPS = 1e-5


LOCAL_HEADS, LOCAL_WINDOW, LOCAL_DILATION = 32, 8, 2
NPRE = 10
AHEAD = 4
BW_AT = 12
WO_AT = 13
LAG_A, LAG_B, LAG_F, LAG_E = 4, 3, 1, 3
UNROLL = 2
PADN = 8
PUNROLL = 1
FIRST = 1


def _ln(xf):
    m = jnp.mean(xf, axis=-1, keepdims=True)
    d = xf - m
    v = jnp.mean(d * d, axis=-1, keepdims=True)
    return d * lax.rsqrt(v + EPS)


def _dot(a, b):
    return jnp.dot(a, b, preferred_element_type=F32)


def _dot_nt(a, b):
    return lax.dot_general(a, b, NT_DIMS, preferred_element_type=F32)


def _unpack(w32):
    return pltpu.bitcast(w32, BF16)


def _kernel(x_hbm, mem0_ref, wq_hbm, wk_hbm, wv_hbm, wo_hbm, bw_hbm, bo_hbm, out_hbm,
            r_ref, h_ref, o_ref, bwp_ref, bop_ref, qb_ref, kb_ref, vb_ref, acc_ref,
            sq_ref, sk_ref, sv_ref, wq_ref, wk_ref, wv_ref, wo_ref, bw_ref, bo_ref,
            hpre_ref, pq_ref, pk_ref, pv_ref, tr_ref, sems, psems,
            *, S, D, H, DH, M, SEG):
    BH, BW, BDIL = LOCAL_HEADS, LOCAL_WINDOW, LOCAL_DILATION
    NS = S // SEG
    NP = H // 2
    PW = 2 * DH
    T1, T3, T4 = 2 * M, 2 * M + SEG, 2 * M + 2 * SEG
    NK = T4 + T1
    PAD = 3
    BDH = D // BH
    HALO = 16
    NT = D // 128
    a_scale = DH ** -0.5
    b_scale = BDH ** -0.5
    XH = (NPRE + 1) * SEG

    cp_bw = pltpu.make_async_copy(bw_hbm, bw_ref, sems.at[0])
    cp_bo = pltpu.make_async_copy(bo_hbm, bo_ref, sems.at[1])
    cp_xh = pltpu.make_async_copy(x_hbm.at[0:XH], r_ref.at[PAD * SEG:PAD * SEG + XH], sems.at[2])
    cp_xt = pltpu.make_async_copy(x_hbm.at[XH:S], r_ref.at[PAD * SEG + XH:PAD * SEG + S], sems.at[3])
    cp_wo = pltpu.make_async_copy(wo_hbm, wo_ref, sems.at[4])

    def pair_copies(p):
        rows = pl.ds(pl.multiple_of(p * PW, PW), PW)
        return [pltpu.make_async_copy(w.at[rows], s.at[rows], psems.at[p])
                for w, s in ((wq_hbm, sq_ref), (wk_hbm, sk_ref), (wv_hbm, sv_ref))]

    def seg(i):
        return pl.ds(pl.multiple_of((i + PAD) * SEG, SEG), SEG)

    def out_copy(i):
        return pltpu.make_async_copy(
            r_ref.at[seg(i)], out_hbm.at[pl.ds(pl.multiple_of(i * SEG, SEG), SEG)], sems.at[5])

    cp_xh.start()
    for p in range(FIRST):
        for cp in pair_copies(p):
            cp.start()

    r_ref[0:PAD * SEG, :] = jnp.zeros((PAD * SEG, D), BF16)
    r_ref[(PAD + NS) * SEG:(2 * PAD + NS) * SEG, :] = jnp.zeros((PAD * SEG, D), BF16)
    qb_ref[...] = jnp.zeros(qb_ref.shape, F32)
    kb_ref[...] = jnp.zeros(kb_ref.shape, F32)
    vb_ref[...] = jnp.zeros(vb_ref.shape, F32)
    mem0 = mem0_ref[...].astype(F32)
    mem00 = jnp.concatenate([mem0, mem0], axis=0)
    h_ref[0, 0:T1, :] = mem00.astype(BF16)
    cp_xh.wait()
    for p in range(FIRST, AHEAD):
        for cp in pair_copies(p):
            cp.start()
    hpre_ref[...] = _ln(r_ref[PAD * SEG:(PAD + NPRE) * SEG, :].astype(F32)).astype(BF16)

    def pair_prologue(p, _):
        for cp in pair_copies(p):
            cp.wait()

        @pl.when(p + AHEAD < NP)
        def _():
            for cp in pair_copies(p + AHEAD):
                cp.start()

        @pl.when(p == BW_AT)
        def _():
            cp_bw.start()
            cp_bo.start()

        @pl.when(p == WO_AT)
        def _():
            cp_wo.start()

        rows = pl.ds(pl.multiple_of(p * PW, PW), PW)
        cols = pl.ds(pl.multiple_of(p * PW, 128), PW)
        hp = hpre_ref[0:(NPRE - 2) * SEG, :]
        for s_ref, w_ref, p_ref in ((sq_ref, wq_ref, pq_ref), (sk_ref, wk_ref, pk_ref),
                                    (sv_ref, wv_ref, pv_ref)):
            w = s_ref[rows, :]
            p_ref[0:(NPRE - 2) * SEG, cols] = _dot_nt(hp, w).astype(BF16)
            w_ref[:, cols] = pltpu.bitcast(w.T, I32)
        return 0

    lax.fori_loop(0, NP, pair_prologue, 0, unroll=PUNROLL)

    def gather_rows(base):
        return jnp.concatenate(
            [tr_ref[pl.ds(base + j, BH, stride=BDH), :] for j in range(BDH)], axis=0)

    cp_bw.wait()
    cp_bo.wait()
    tr_ref[3 * D:3 * D + BH, :] = jnp.zeros((BH, 128), F32)
    for kt in range(NT):
        tr_ref[0:3 * D, :] = bw_ref[kt * 128:(kt + 1) * 128, :].T.astype(F32)
        for i in range(3):
            g = gather_rows(i * D).astype(BF16).T
            bwp_ref[kt * 64:(kt + 1) * 64, i * D:(i + 1) * D] = pltpu.bitcast(g, I32)
    for lt in range(NT):
        tr_ref[0:D, :] = bo_ref[:, lt * 128:(lt + 1) * 128].astype(F32)
        bop_ref[:, lt * 128:(lt + 1) * 128] = pltpu.bitcast(gather_rows(0).astype(BF16), I32)

    def b_seg(t, l):
        return t - 1 - 2 * l

    def b_local_attn(t, slots):
        blocks = []
        for l in slots:
            for rb in range(SEG // 8):
                pos = lax.broadcasted_iota(I32, (8, 128), 0) + (b_seg(t, l) * SEG + rb * 8)
                qs = [qb_ref[l, c, rb * 8:rb * 8 + 8, :] for c in range(NT)]
                logits = []
                for w in range(BW):
                    r0 = HALO - BDIL * w + rb * 8
                    a = None
                    for c in range(NT):
                        pr = qs[c] * kb_ref[l, c, r0:r0 + 8, :]
                        a = pr if a is None else a + pr
                    a = a + pltpu.roll(a, 64, 1)
                    a = a + pltpu.roll(a, 32, 1)
                    logits.append(jnp.where(pos >= BDIL * w, a, NEG))
                mx = logits[0]
                for w in range(1, BW):
                    mx = jnp.maximum(mx, logits[w])
                es = [jnp.exp(a - mx) for a in logits]
                sm = es[0]
                for w in range(1, BW):
                    sm = sm + es[w]
                inv = 1.0 / sm
                aws = [e * inv for e in es]
                tiles = []
                for c in range(NT):
                    ob = None
                    for w in range(BW):
                        r0 = HALO - BDIL * w + rb * 8
                        term = aws[w] * vb_ref[l, c, r0:r0 + 8, :]
                        ob = term if ob is None else ob + term
                    tiles.append(ob)
                blocks.append(jnp.concatenate(tiles, axis=1))
        return jnp.concatenate(blocks, axis=0).astype(BF16)

    def b_out(t, slots, ob):
        bout = _dot(ob, _unpack(bop_ref[...]))
        news = []
        for i, l in enumerate(slots):
            sg = seg(b_seg(t, l))
            new = (r_ref[sg, :].astype(F32) + bout[i * SEG:(i + 1) * SEG]).astype(BF16)
            r_ref[sg, :] = new
            news.append(new)
        return news

    def b_qkv(slots, xs):
        hb = jnp.concatenate([_ln(x.astype(F32)) for x in xs], axis=0).astype(BF16)
        qkv = _dot(hb, _unpack(bwp_ref[...]))
        for i, l in enumerate(slots):
            rows = slice(i * SEG, (i + 1) * SEG)
            for c in range(NT):
                c0 = c * 128
                qb_ref[l, c] = qkv[rows, c0:c0 + 128] * b_scale
                kb_ref[l, c, 0:HALO, :] = kb_ref[l, c, SEG:SEG + HALO, :]
                vb_ref[l, c, 0:HALO, :] = vb_ref[l, c, SEG:SEG + HALO, :]
                kb_ref[l, c, HALO:HALO + SEG, :] = qkv[rows, D + c0:D + c0 + 128]
                vb_ref[l, c, HALO:HALO + SEG, :] = qkv[rows, 2 * D + c0:2 * D + c0 + 128]

    def softmax(s, mask):
        s = jnp.where(mask, s * a_scale, NEG)
        mx = jnp.max(s, axis=-1, keepdims=True)
        e = jnp.exp(s - mx)
        sm = jnp.sum(e, axis=-1, keepdims=True)
        return e * (1.0 / sm)

    def split_lo_hi(z):
        rows = z.shape[0]
        lo32 = jnp.where(lax.broadcasted_iota(I32, (rows // 2, 128), 1) < 64, I32(-1), I32(0))
        zi = pltpu.bitcast(z, I32)
        return pltpu.bitcast(zi & lo32, BF16), pltpu.bitcast(zi & ~lo32, BF16)

    def step(t, kind, lag):
        if kind == "head":
            @pl.when(t == NS)
            def _():
                for i in range(PADN):
                    acc_ref[...] = _dot(hpre_ref[0:T4, :], _unpack(wq_ref[:, i * D:(i + 2) * D]))[:, 0:D]
        slot = lax.rem(t, 2)
        nslot = 1 - slot
        both = kind in ("ramp", "full")
        lay = 0 if kind == "head" else 1
        RW = T4 if both else T3
        if kind == "full":
            hrows = h_ref[slot]
        elif kind == "head":
            arows = pl.ds(pl.multiple_of((NPRE - 2 + t) * SEG, SEG), SEG)
            hrows = jnp.concatenate([h_ref[slot, 0:T1, :], hpre_ref[arows, :]], axis=0)
        else:
            hrows = jnp.concatenate([h_ref[slot, 0:T1, :], h_ref[slot, T3:T4, :]], axis=0)
        b_attn_slots = {"head": (0,), "ramp": (0, 1), "full": (0, 1), "tail": (0, 1)}[kind]
        b_qkv_slots = {"head": (0,), "ramp": (0, 1), "full": (0, 1), "tail": (1,)}[kind]

        ri = lax.broadcasted_iota(I32, (RW, NK), 0)
        ci = lax.broadcasted_iota(I32, (RW, NK), 1)
        if both:
            def layer(i):
                return jnp.where(i < M, 0, jnp.where(i < T1, 1, jnp.where(i < T3, 0, 1)))

            def allowed(kidx, kvalid):
                return kvalid & (layer(ri) == layer(kidx)) & ((ri < T1) | (kidx < T1) | (ri >= kidx))
            mask0 = allowed(ci, ci < T4)
            nat1 = jnp.where(ci < T3, ci - T1 + T3, jnp.where(ci < T4, ci - T3 + T1, ci - T4))
            mask1 = allowed(nat1, ci >= T1)

            def shared_w(z):
                zl, zh = split_lo_hi(z)
                w1 = jnp.concatenate([zl[0:T3], zh[T1:T3], zh[0:T1]], axis=0)
                w3 = jnp.concatenate([zl[0:T1], zh[T3:T4], zl[T3:T4], zh[0:T1]], axis=0)
                return w1, w3

            def h0_rows(z):
                return jnp.concatenate([z, z[0:T1]], axis=0)

            def h1_rows(z):
                return jnp.concatenate([z[0:T1], z[T3:T4], z[T1:T3], z[0:T1]], axis=0)

            def shared(dot, lhs, ws):
                y1 = dot(lhs[0:T3], ws[0])
                y3 = dot(jnp.concatenate([lhs[0:T1], lhs[T3:T4]], axis=0), ws[1])
                return jnp.concatenate([y1[0:M], y3[M:T1], y1[T1:T3], y3[T1:T3]], axis=0)
        else:
            def allowed(kidx, kvalid):
                kok = kvalid & ((kidx >= T1) | (kidx // M == lay))
                return kok & ((ri < T1) | (kidx < T1) | (ri >= kidx))
            mask0 = allowed(ci, ci < T3)
            nat1 = jnp.where(ci < T4, ci - T3 + T1, ci - T4)
            mask1 = allowed(nat1, ci >= T3)

            def shared_w(z):
                zl, zh = split_lo_hi(z)
                return (jnp.concatenate([zl, zh[T1:T3], zh[0:T1]], axis=0),)

            def h0_rows(z):
                return jnp.concatenate([z, z], axis=0)

            def h1_rows(z):
                return jnp.concatenate([z, z[T1:T3], z[0:T1]], axis=0)

            def shared(dot, lhs, ws):
                return dot(lhs, ws[0])

        def proj(w_ref, pre_ref, p):
            c0 = p * PW
            y = _dot(hrows, _unpack(w_ref[:, c0:c0 + PW])).astype(BF16)
            if kind in ("full", "tail"):
                return y
            pre = pre_ref[pl.ds(pl.multiple_of(t * SEG, SEG), SEG), c0:c0 + PW]
            if kind == "ramp":
                return jnp.concatenate([y[0:T1], pre, y[T1:T3]], axis=0)
            pre_ref[arows, c0:c0 + PW] = y[T1:T3]
            return jnp.concatenate([y[0:T1], pre], axis=0)

        def qk(q, k):
            qA, qB, qC = q[:, 0:128], q[:, 128:256], q[:, 256:384]
            sa = _dot_nt(qA, h0_rows(k[:, 0:128]))
            sc = _dot_nt(qC, h1_rows(k[:, 256:384]))
            x = shared(_dot_nt, qB, shared_w(k[:, 128:256]))
            return sa + x, sc + x

        def pv(p, s0, s1, v):
            c0 = p * PW
            p0 = softmax(s0, mask0)
            p1 = softmax(s1, mask1)
            pm = (p0 + p1).astype(BF16)
            oa = _dot(p0.astype(BF16), h0_rows(v[:, 0:128]))
            oc = _dot(p1.astype(BF16), h1_rows(v[:, 256:384]))
            ob_ = shared(_dot, pm, shared_w(v[:, 128:256]))
            o_ref[0:RW, c0:c0 + 128] = oa.astype(BF16)
            o_ref[0:RW, c0 + 128:c0 + 256] = ob_.astype(BF16)
            o_ref[0:RW, c0 + 256:c0 + 384] = oc.astype(BF16)

        def out_chunk(c0, c1):
            return _dot(o_ref[0:RW, c0 * PW:c1 * PW], wo_ref[c0 * PW:c1 * PW, :])

        ob = b_local_attn(t, b_attn_slots)

        qs, ks, vs, ss = {}, {}, {}, {}
        cuts = [0, (NP + 1 - lag) // 2] + [NP - lag + s for s in range(1, lag)]
        for p in range(NP + lag):
            if 1 <= p <= NP:
                ss[p - 1] = qk(qs.pop(p - 1), ks.pop(p - 1))
            if p < NP:
                qs[p] = proj(wq_ref, pq_ref, p)
                ks[p] = proj(wk_ref, pk_ref, p)
            elif p == NP:
                if kind == "head":
                    @pl.when(t == 0)
                    def _():
                        cp_wo.wait()
                        cp_xt.start()
                acc_ref[0:RW] = out_chunk(cuts[0], cuts[1])
            else:
                acc_ref[0:RW] += out_chunk(cuts[p - NP], cuts[p - NP + 1])
            if p >= lag:
                pv(p - lag, *ss.pop(p - lag), vs.pop(p - lag))
            if p < NP:
                vs[p] = proj(wv_ref, pv_ref, p)
        aout = acc_ref[0:RW] + out_chunk(cuts[lag], NP)

        def add_residual(i, rows):
            new = (r_ref[seg(i), :].astype(F32) + aout[rows]).astype(BF16)
            r_ref[seg(i), :] = new
            return new

        if kind == "head":
            xs = [add_residual(t, slice(T1, T3))]
        elif kind == "tail":
            xs = [add_residual(t - 2, slice(T1, T3))]
        else:
            xs = [add_residual(t, slice(T1, T3)), add_residual(t - 2, slice(T3, T4))]
        mrow = lax.broadcasted_iota(I32, (T1, D), 0)
        keep = (mrow < M) | (t >= 2)
        h_ref[nslot, 0:T1, :] = jnp.where(keep, aout[0:T1], mem00).astype(BF16)
        if kind != "tail":
            h_ref[nslot, T1:T3, :] = _ln(r_ref[seg(t + 1), :].astype(F32)).astype(BF16)

        news = b_out(t, b_attn_slots, ob)
        h_ref[nslot, T3:T4, :] = _ln(news[0].astype(F32)).astype(BF16)
        b_qkv(b_qkv_slots, xs)
        if kind != "head":
            @pl.when(t >= 3)
            def _():
                out_copy(t - 3).start()

    def loop(lo, hi, kind, lag, unroll=1):
        assert (hi - lo) % unroll == 0

        def body(i, _):
            for u in range(unroll):
                step(lo + i * unroll + u, kind, lag)
            return 0
        lax.fori_loop(0, (hi - lo) // unroll, body, 0)

    loop(0, 2, "head", LAG_A)
    loop(2, NPRE, "ramp", LAG_B)
    cp_xt.wait()
    loop(NPRE, NS, "full", LAG_F, UNROLL)
    loop(NS, NS + 2, "tail", LAG_E)
    b_out(NS + 2, (1,), b_local_attn(NS + 2, (1,)))
    out_copy(NS - 1).start()
    pltpu.make_async_copy(r_ref.at[PAD * SEG:(PAD + NS) * SEG], out_hbm, sems.at[5]).wait()


@functools.partial(jax.jit, static_argnames=("A_seg_len",))
def pallas_interleave_layers__memory_aug_recurrent_mem_tr__sliding_local_dilated__prompt_kernel(A_x, A_mem0, A_Wq, A_Wk, A_Wv, A_Wo, A_seg_len, B_x, B_wqkv, B_wo):
    del B_x
    B, S, D = A_x.shape
    M = A_mem0.shape[1]
    _, H, DH = A_Wq.shape
    SEG = A_seg_len
    HD = H * DH
    x = A_x.reshape(S, D)
    mem0 = A_mem0.reshape(M, D)
    wq = jnp.transpose(A_Wq, (1, 2, 0)).reshape(HD, D)
    wk = jnp.transpose(A_Wk, (1, 2, 0)).reshape(HD, D)
    wv = jnp.transpose(A_Wv, (1, 2, 0)).reshape(HD, D)
    wo = A_Wo.reshape(HD, D)
    R2 = 2 * M + 2 * SEG
    kern = functools.partial(_kernel, S=S, D=D, H=H, DH=DH, M=M, SEG=SEG)
    hbm = pl.BlockSpec(memory_space=pl.ANY)
    out = pl.pallas_call(
        kern,
        out_shape=jax.ShapeDtypeStruct((S, D), BF16),
        in_specs=[hbm, pl.BlockSpec(memory_space=pltpu.VMEM)] + [hbm] * 6,
        out_specs=hbm,
        scratch_shapes=[
            pltpu.VMEM((S + 6 * SEG, D), BF16),
            pltpu.VMEM((2, R2, D), BF16),
            pltpu.VMEM((R2, HD), BF16),
            pltpu.VMEM((D // 2, 3 * D), I32),
            pltpu.VMEM((D // 2, D), I32),
            pltpu.VMEM((2, D // 128, SEG, 128), F32),
            pltpu.VMEM((2, D // 128, 16 + SEG, 128), F32),
            pltpu.VMEM((2, D // 128, 16 + SEG, 128), F32),
            pltpu.VMEM((R2, D), F32),
            pltpu.VMEM((HD, D), BF16),
            pltpu.VMEM((HD, D), BF16),
            pltpu.VMEM((HD, D), BF16),
            pltpu.VMEM((D // 2, HD), I32),
            pltpu.VMEM((D // 2, HD), I32),
            pltpu.VMEM((D // 2, HD), I32),
            pltpu.VMEM((HD, D), BF16),
            pltpu.VMEM((D, 3 * D), BF16),
            pltpu.VMEM((D, D), BF16),
            pltpu.VMEM((NPRE * SEG, D), BF16),
            pltpu.VMEM((NPRE * SEG, HD), BF16),
            pltpu.VMEM((NPRE * SEG, HD), BF16),
            pltpu.VMEM((NPRE * SEG, HD), BF16),
            pltpu.VMEM((3 * D + LOCAL_HEADS, 128), F32),
            pltpu.SemaphoreType.DMA((6,)),
            pltpu.SemaphoreType.DMA((H // 2,)),
        ],
        compiler_params=pltpu.CompilerParams(
            vmem_limit_bytes=120 * 2**20,
            flags={"XLA_TPU_EVENLY_DISTRIBUTE_CRITICAL_NODES": True}),
    )(x, mem0, wq, wk, wv, wo, B_wqkv, B_wo)
    return out.reshape(B, S, D)
```

```python
import functools

import jax
import jax.numpy as jnp
from jax import lax
from jax.experimental import pallas as pl
from jax.experimental.pallas import tpu as pltpu

F32 = jnp.float32
BF16 = jnp.bfloat16
I32 = jnp.int32
NT_DIMS = (((1,), (1,)), ((), ()))
NEG = -1e9
EPS = 1e-5


LOCAL_HEADS, LOCAL_WINDOW, LOCAL_DILATION = 32, 8, 2
NPRE = 10
AHEAD = 4
BW_AT = 12
WO_AT = 13
LAG_A, LAG_B, LAG_F, LAG_E = 4, 3, 1, 3
UNROLL = 2
PADN = 8
FIRST = 1


def _ln(xf):
    m = jnp.mean(xf, axis=-1, keepdims=True)
    d = xf - m
    v = jnp.mean(d * d, axis=-1, keepdims=True)
    return d * lax.rsqrt(v + EPS)


def _recip(x):
    r = pl.reciprocal(x, approx=True)
    return r * (2.0 - x * r)


def _dot(a, b):
    return jnp.dot(a, b, preferred_element_type=F32)


def _dot_nt(a, b):
    return lax.dot_general(a, b, NT_DIMS, preferred_element_type=F32)


def _unpack(w32):
    return pltpu.bitcast(w32, BF16)


def _pack(x):
    return pltpu.bitcast(x.astype(BF16), I32)


def _prow(start, size):
    return pl.ds(start // 2, size // 2) if isinstance(start, int) else pl.ds(pl.multiple_of(start // 2, 8), size // 2)


def _kernel(x_hbm, mem0_ref, wq_hbm, wk_hbm, wv_hbm, wo_hbm, bw_hbm, bo_hbm, out_hbm,
            r_ref, h_ref, o_ref, bwp_ref, bop_ref, qb_ref, kb_ref, vb_ref, acc_ref,
            sq_ref, sk_ref, sv_ref, wq_ref, wk_ref, wv_ref, wo_ref, bw_ref, bo_ref,
            hpre_ref, pq_ref, pk_ref, pv_ref, tr_ref, sems, psems,
            *, S, D, H, DH, M, SEG):
    BH, BW, BDIL = LOCAL_HEADS, LOCAL_WINDOW, LOCAL_DILATION
    NS = S // SEG
    NP = H // 2
    PW = 2 * DH
    T1, T3, T4 = 2 * M, 2 * M + SEG, 2 * M + 2 * SEG
    NK = T4 + T1
    PAD = 3
    BDH = D // BH
    HALO = 16
    NT = D // 128
    a_scale = DH ** -0.5
    b_scale = BDH ** -0.5
    XH = (NPRE + 1) * SEG

    cp_bw = pltpu.make_async_copy(bw_hbm, bw_ref, sems.at[0])
    cp_bo = pltpu.make_async_copy(bo_hbm, bo_ref, sems.at[1])
    cp_xh = pltpu.make_async_copy(x_hbm.at[0:XH], r_ref.at[PAD * SEG:PAD * SEG + XH], sems.at[2])
    cp_xt = pltpu.make_async_copy(x_hbm.at[XH:S], r_ref.at[PAD * SEG + XH:PAD * SEG + S], sems.at[3])
    cp_wo = pltpu.make_async_copy(wo_hbm, wo_ref, sems.at[4])

    def pair_copies(p):
        rows = pl.ds(pl.multiple_of(p * PW, PW), PW)
        return [pltpu.make_async_copy(w.at[rows], s.at[rows], psems.at[p])
                for w, s in ((wq_hbm, sq_ref), (wk_hbm, sk_ref), (wv_hbm, sv_ref))]

    def seg(i):
        return pl.ds(pl.multiple_of((i + PAD) * SEG, SEG), SEG)

    def out_copy(i):
        return pltpu.make_async_copy(
            r_ref.at[seg(i)], out_hbm.at[pl.ds(pl.multiple_of(i * SEG, SEG), SEG)], sems.at[5])

    cp_xh.start()
    for p in range(FIRST):
        for cp in pair_copies(p):
            cp.start()

    r_ref[0:PAD * SEG, :] = jnp.zeros((PAD * SEG, D), BF16)
    r_ref[(PAD + NS) * SEG:(2 * PAD + NS) * SEG, :] = jnp.zeros((PAD * SEG, D), BF16)
    qb_ref[...] = jnp.zeros(qb_ref.shape, F32)
    kb_ref[...] = jnp.zeros(kb_ref.shape, F32)
    vb_ref[...] = jnp.zeros(vb_ref.shape, F32)
    mem0 = mem0_ref[...].astype(F32)
    mem00 = jnp.concatenate([mem0, mem0], axis=0)
    h_ref[0, _prow(0, T1), :] = _pack(mem00)
    cp_xh.wait()
    for p in range(FIRST, AHEAD):
        for cp in pair_copies(p):
            cp.start()
    hpre_ref[...] = _pack(_ln(r_ref[PAD * SEG:(PAD + NPRE) * SEG, :].astype(F32)))

    def pair_prologue(p, _):
        for cp in pair_copies(p):
            cp.wait()

        @pl.when(p + AHEAD < NP)
        def _():
            for cp in pair_copies(p + AHEAD):
                cp.start()

        @pl.when(p == BW_AT)
        def _():
            cp_bw.start()
            cp_bo.start()

        @pl.when(p == WO_AT)
        def _():
            cp_wo.start()

        rows = pl.ds(pl.multiple_of(p * PW, PW), PW)
        cols = pl.ds(pl.multiple_of(p * PW, 128), PW)
        hp = _unpack(hpre_ref[_prow(0, (NPRE - 2) * SEG), :])
        for s_ref, w_ref, p_ref in ((sq_ref, wq_ref, pq_ref), (sk_ref, wk_ref, pk_ref),
                                    (sv_ref, wv_ref, pv_ref)):
            w = s_ref[rows, :]
            p_ref[_prow(0, (NPRE - 2) * SEG), cols] = _pack(_dot_nt(hp, w))
            w_ref[:, cols] = pltpu.bitcast(w.T, I32)
        return 0

    lax.fori_loop(0, NP, pair_prologue, 0)

    def gather_rows(base):
        return jnp.concatenate(
            [tr_ref[pl.ds(base + j, BH, stride=BDH), :] for j in range(BDH)], axis=0)

    cp_bw.wait()
    cp_bo.wait()
    tr_ref[3 * D:3 * D + BH, :] = jnp.zeros((BH, 128), F32)
    for kt in range(NT):
        tr_ref[0:3 * D, :] = bw_ref[kt * 128:(kt + 1) * 128, :].T.astype(F32)
        for i in range(3):
            g = gather_rows(i * D).astype(BF16).T
            bwp_ref[kt * 64:(kt + 1) * 64, i * D:(i + 1) * D] = pltpu.bitcast(g, I32)
    for lt in range(NT):
        tr_ref[0:D, :] = bo_ref[:, lt * 128:(lt + 1) * 128].astype(F32)
        bop_ref[:, lt * 128:(lt + 1) * 128] = pltpu.bitcast(gather_rows(0).astype(BF16), I32)

    def b_seg(t, l):
        return t - 1 - 2 * l

    def b_local_attn(t, slots, masked=True):
        blocks = []
        for l in slots:
            for rb in range(SEG // 8):
                pos = lax.broadcasted_iota(I32, (8, 128), 0) + (b_seg(t, l) * SEG + rb * 8)
                qs = [qb_ref[l, c, rb * 8:rb * 8 + 8, :] for c in range(NT)]
                logits = []
                for w in range(BW):
                    r0 = HALO - BDIL * w + rb * 8
                    a = None
                    for c in range(NT):
                        pr = qs[c] * kb_ref[l, c, r0:r0 + 8, :]
                        a = pr if a is None else a + pr
                    a = a + pltpu.roll(a, 64, 1)
                    a = a + pltpu.roll(a, 32, 1)
                    logits.append(jnp.where(pos >= BDIL * w, a, NEG) if (masked and BDIL * w > rb * 8) else a)
                mx = logits[0]
                for w in range(1, BW):
                    mx = jnp.maximum(mx, logits[w])
                es = [jnp.exp(a - mx) for a in logits]
                sm = es[0]
                for w in range(1, BW):
                    sm = sm + es[w]
                inv = _recip(sm)
                aws = [e * inv for e in es]
                tiles = []
                for c in range(NT):
                    ob = None
                    for w in range(BW):
                        r0 = HALO - BDIL * w + rb * 8
                        term = aws[w] * vb_ref[l, c, r0:r0 + 8, :]
                        ob = term if ob is None else ob + term
                    tiles.append(ob)
                blocks.append(jnp.concatenate(tiles, axis=1))
        return jnp.concatenate(blocks, axis=0).astype(BF16)

    def b_out(t, slots, ob):
        bout = _dot(ob, _unpack(bop_ref[...]))
        news = []
        for i, l in enumerate(slots):
            sg = seg(b_seg(t, l))
            new = (r_ref[sg, :].astype(F32) + bout[i * SEG:(i + 1) * SEG]).astype(BF16)
            r_ref[sg, :] = new
            news.append(new)
        return news

    def b_qkv(slots, xs):
        hb = jnp.concatenate([_ln(x.astype(F32)) for x in xs], axis=0).astype(BF16)
        qkv = _dot(hb, _unpack(bwp_ref[...]))
        for i, l in enumerate(slots):
            rows = slice(i * SEG, (i + 1) * SEG)
            for c in range(NT):
                c0 = c * 128
                qb_ref[l, c] = qkv[rows, c0:c0 + 128] * b_scale
                kb_ref[l, c, 0:HALO, :] = kb_ref[l, c, SEG:SEG + HALO, :]
                vb_ref[l, c, 0:HALO, :] = vb_ref[l, c, SEG:SEG + HALO, :]
                kb_ref[l, c, HALO:HALO + SEG, :] = qkv[rows, D + c0:D + c0 + 128]
                vb_ref[l, c, HALO:HALO + SEG, :] = qkv[rows, 2 * D + c0:2 * D + c0 + 128]

    def softmax(s, mask):
        s = jnp.where(mask, s * a_scale, NEG)
        mx = jnp.max(s, axis=-1, keepdims=True)
        e = jnp.exp(s - mx)
        return e * _recip(jnp.sum(e, axis=-1, keepdims=True))

    def split_lo_hi(z):
        rows = z.shape[0]
        lo32 = jnp.where(lax.broadcasted_iota(I32, (rows // 2, 128), 1) < 64, I32(-1), I32(0))
        zi = pltpu.bitcast(z, I32)
        return pltpu.bitcast(zi & lo32, BF16), pltpu.bitcast(zi & ~lo32, BF16)

    def step(t, kind, lag):
        if kind == "head":
            @pl.when(t == NS)
            def _():
                for i in range(PADN):
                    acc_ref[...] = _dot(_unpack(hpre_ref[_prow(0, T4), :]), _unpack(wq_ref[:, i * D:(i + 2) * D]))[:, 0:D]
        slot = lax.rem(t, 2)
        nslot = 1 - slot
        both = kind in ("ramp", "full")
        lay = 0 if kind == "head" else 1
        RW = T4 if both else T3
        if kind == "full":
            hrows = _unpack(h_ref[slot])
        elif kind == "head":
            arows = _prow((NPRE - 2 + t) * SEG, SEG)
            hrows = _unpack(jnp.concatenate([h_ref[slot, _prow(0, T1), :], hpre_ref[arows, :]], axis=0))
        else:
            hrows = _unpack(jnp.concatenate([h_ref[slot, _prow(0, T1), :], h_ref[slot, _prow(T3, SEG), :]], axis=0))
        b_attn_slots = {"head": (0,), "ramp": (0, 1), "full": (0, 1), "tail": (0, 1)}[kind]
        b_qkv_slots = {"head": (0,), "ramp": (0, 1), "full": (0, 1), "tail": (1,)}[kind]

        ri = lax.broadcasted_iota(I32, (RW, NK), 0)
        ci = lax.broadcasted_iota(I32, (RW, NK), 1)
        if both:
            def layer(i):
                return jnp.where(i < M, 0, jnp.where(i < T1, 1, jnp.where(i < T3, 0, 1)))

            def allowed(kidx, kvalid):
                return kvalid & (layer(ri) == layer(kidx)) & ((ri < T1) | (kidx < T1) | (ri >= kidx))
            mask0 = allowed(ci, ci < T4)
            nat1 = jnp.where(ci < T3, ci - T1 + T3, jnp.where(ci < T4, ci - T3 + T1, ci - T4))
            mask1 = allowed(nat1, ci >= T1)

            def shared_w(z):
                zl, zh = split_lo_hi(z)
                w1 = jnp.concatenate([zl[0:T3], zh[T1:T3], zh[0:T1]], axis=0)
                w3 = jnp.concatenate([zl[0:T1], zh[T3:T4], zl[T3:T4], zh[0:T1]], axis=0)
                return w1, w3

            def h0_rows(z):
                return jnp.concatenate([z, z[0:T1]], axis=0)

            def h1_rows(z):
                return jnp.concatenate([z[0:T1], z[T3:T4], z[T1:T3], z[0:T1]], axis=0)

            def shared(dot, lhs, ws):
                y1 = dot(lhs[0:T3], ws[0])
                y3 = dot(jnp.concatenate([lhs[0:T1], lhs[T3:T4]], axis=0), ws[1])
                return jnp.concatenate([y1[0:M], y3[M:T1], y1[T1:T3], y3[T1:T3]], axis=0)
        else:
            def allowed(kidx, kvalid):
                kok = kvalid & ((kidx >= T1) | (kidx // M == lay))
                return kok & ((ri < T1) | (kidx < T1) | (ri >= kidx))
            mask0 = allowed(ci, ci < T3)
            nat1 = jnp.where(ci < T4, ci - T3 + T1, ci - T4)
            mask1 = allowed(nat1, ci >= T3)

            def shared_w(z):
                zl, zh = split_lo_hi(z)
                return (jnp.concatenate([zl, zh[T1:T3], zh[0:T1]], axis=0),)

            def h0_rows(z):
                return jnp.concatenate([z, z], axis=0)

            def h1_rows(z):
                return jnp.concatenate([z, z[T1:T3], z[0:T1]], axis=0)

            def shared(dot, lhs, ws):
                return dot(lhs, ws[0])

        def proj(w_ref, pre_ref, p):
            c0 = p * PW
            y = _dot(hrows, _unpack(w_ref[:, c0:c0 + PW])).astype(BF16)
            if kind in ("full", "tail"):
                return y
            pre = _unpack(pre_ref[_prow(t * SEG, SEG), c0:c0 + PW])
            if kind == "ramp":
                return jnp.concatenate([y[0:T1], pre, y[T1:T3]], axis=0)
            pre_ref[arows, c0:c0 + PW] = pltpu.bitcast(y[T1:T3], I32)
            return jnp.concatenate([y[0:T1], pre], axis=0)

        def qk(q, k):
            qA, qB, qC = q[:, 0:128], q[:, 128:256], q[:, 256:384]
            sa = _dot_nt(qA, h0_rows(k[:, 0:128]))
            sc = _dot_nt(qC, h1_rows(k[:, 256:384]))
            x = shared(_dot_nt, qB, shared_w(k[:, 128:256]))
            return sa + x, sc + x

        def pv(p, s0, s1, v):
            c0 = p * PW
            p0 = softmax(s0, mask0)
            p1 = softmax(s1, mask1)
            pm = (p0 + p1).astype(BF16)
            oa = _dot(p0.astype(BF16), h0_rows(v[:, 0:128]))
            oc = _dot(p1.astype(BF16), h1_rows(v[:, 256:384]))
            ob_ = shared(_dot, pm, shared_w(v[:, 128:256]))
            o_ref[_prow(0, RW), c0:c0 + 128] = _pack(oa)
            o_ref[_prow(0, RW), c0 + 128:c0 + 256] = _pack(ob_)
            o_ref[_prow(0, RW), c0 + 256:c0 + 384] = _pack(oc)

        def out_chunk(c0, c1):
            return _dot(_unpack(o_ref[_prow(0, RW), c0 * PW:c1 * PW]), wo_ref[c0 * PW:c1 * PW, :])

        ob = b_local_attn(t, b_attn_slots, masked=kind in ("head", "ramp"))

        qs, ks, vs, ss = {}, {}, {}, {}
        cuts = [0, (NP + 1 - lag) // 2] + [NP - lag + s for s in range(1, lag)]
        for p in range(NP + lag):
            if 1 <= p <= NP:
                ss[p - 1] = qk(qs.pop(p - 1), ks.pop(p - 1))
            if p < NP:
                qs[p] = proj(wq_ref, pq_ref, p)
                ks[p] = proj(wk_ref, pk_ref, p)
            elif p == NP:
                if kind == "head":
                    @pl.when(t == 0)
                    def _():
                        cp_wo.wait()
                        cp_xt.start()
                acc_ref[0:RW] = out_chunk(cuts[0], cuts[1])
            else:
                acc_ref[0:RW] += out_chunk(cuts[p - NP], cuts[p - NP + 1])
            if p >= lag:
                pv(p - lag, *ss.pop(p - lag), vs.pop(p - lag))
            if p < NP:
                vs[p] = proj(wv_ref, pv_ref, p)
        aout = acc_ref[0:RW] + out_chunk(cuts[lag], NP)

        def add_residual(i, rows):
            new = (r_ref[seg(i), :].astype(F32) + aout[rows]).astype(BF16)
            r_ref[seg(i), :] = new
            return new

        if kind == "head":
            xs = [add_residual(t, slice(T1, T3))]
        elif kind == "tail":
            xs = [add_residual(t - 2, slice(T1, T3))]
        else:
            xs = [add_residual(t, slice(T1, T3)), add_residual(t - 2, slice(T3, T4))]
        mrow = lax.broadcasted_iota(I32, (T1, D), 0)
        keep = (mrow < M) | (t >= 2)
        h_ref[nslot, _prow(0, T1), :] = _pack(jnp.where(keep, aout[0:T1], mem00))
        if kind != "tail":
            h_ref[nslot, _prow(T1, SEG), :] = _pack(_ln(r_ref[seg(t + 1), :].astype(F32)))

        news = b_out(t, b_attn_slots, ob)
        h_ref[nslot, _prow(T3, SEG), :] = _pack(_ln(news[0].astype(F32)))
        b_qkv(b_qkv_slots, xs)
        if kind != "head":
            @pl.when(t >= 3)
            def _():
                out_copy(t - 3).start()

    def loop(lo, hi, kind, lag, unroll=1):
        assert (hi - lo) % unroll == 0

        def body(i, _):
            for u in range(unroll):
                step(lo + i * unroll + u, kind, lag)
            return 0
        lax.fori_loop(0, (hi - lo) // unroll, body, 0)

    loop(0, 2, "head", LAG_A)
    loop(2, NPRE, "ramp", LAG_B)
    cp_xt.wait()
    loop(NPRE, NS, "full", LAG_F, UNROLL)
    loop(NS, NS + 2, "tail", LAG_E)
    b_out(NS + 2, (1,), b_local_attn(NS + 2, (1,)))
    out_copy(NS - 1).start()
    pltpu.make_async_copy(r_ref.at[PAD * SEG:(PAD + NS) * SEG], out_hbm, sems.at[5]).wait()


@functools.partial(jax.jit, static_argnames=("A_seg_len",))
def pallas_interleave_layers__memory_aug_recurrent_mem_tr__sliding_local_dilated__prompt_kernel(A_x, A_mem0, A_Wq, A_Wk, A_Wv, A_Wo, A_seg_len, B_x, B_wqkv, B_wo):
    del B_x
    B, S, D = A_x.shape
    M = A_mem0.shape[1]
    _, H, DH = A_Wq.shape
    SEG = A_seg_len
    HD = H * DH
    x = A_x.reshape(S, D)
    mem0 = A_mem0.reshape(M, D)
    wq = jnp.transpose(A_Wq, (1, 2, 0)).reshape(HD, D)
    wk = jnp.transpose(A_Wk, (1, 2, 0)).reshape(HD, D)
    wv = jnp.transpose(A_Wv, (1, 2, 0)).reshape(HD, D)
    wo = A_Wo.reshape(HD, D)
    R2 = 2 * M + 2 * SEG
    kern = functools.partial(_kernel, S=S, D=D, H=H, DH=DH, M=M, SEG=SEG)
    hbm = pl.BlockSpec(memory_space=pl.ANY)
    out = pl.pallas_call(
        kern,
        out_shape=jax.ShapeDtypeStruct((S, D), BF16),
        in_specs=[hbm, pl.BlockSpec(memory_space=pltpu.VMEM)] + [hbm] * 6,
        out_specs=hbm,
        scratch_shapes=[
            pltpu.VMEM((S + 6 * SEG, D), BF16),
            pltpu.VMEM((2, R2 // 2, D), I32),
            pltpu.VMEM((R2 // 2, HD), I32),
            pltpu.VMEM((D // 2, 3 * D), I32),
            pltpu.VMEM((D // 2, D), I32),
            pltpu.VMEM((2, D // 128, SEG, 128), F32),
            pltpu.VMEM((2, D // 128, 16 + SEG, 128), F32),
            pltpu.VMEM((2, D // 128, 16 + SEG, 128), F32),
            pltpu.VMEM((R2, D), F32),
            pltpu.VMEM((HD, D), BF16),
            pltpu.VMEM((HD, D), BF16),
            pltpu.VMEM((HD, D), BF16),
            pltpu.VMEM((D // 2, HD), I32),
            pltpu.VMEM((D // 2, HD), I32),
            pltpu.VMEM((D // 2, HD), I32),
            pltpu.VMEM((HD, D), BF16),
            pltpu.VMEM((D, 3 * D), BF16),
            pltpu.VMEM((D, D), BF16),
            pltpu.VMEM((NPRE * SEG // 2, D), I32),
            pltpu.VMEM((NPRE * SEG // 2, HD), I32),
            pltpu.VMEM((NPRE * SEG // 2, HD), I32),
            pltpu.VMEM((NPRE * SEG // 2, HD), I32),
            pltpu.VMEM((3 * D + LOCAL_HEADS, 128), F32),
            pltpu.SemaphoreType.DMA((6,)),
            pltpu.SemaphoreType.DMA((H // 2,)),
        ],
        compiler_params=pltpu.CompilerParams(
            vmem_limit_bytes=120 * 2**20,
            flags={"XLA_TPU_EVENLY_DISTRIBUTE_CRITICAL_NODES": True}),
    )(x, mem0, wq, wk, wv, wo, B_wqkv, B_wo)
    return out.reshape(B, S, D)
```

```python
import functools

import jax
import jax.numpy as jnp
from jax import lax
from jax.experimental import pallas as pl
from jax.experimental.pallas import tpu as pltpu

F32 = jnp.float32
BF16 = jnp.bfloat16
I32 = jnp.int32
NT_DIMS = (((1,), (1,)), ((), ()))
NEG = -1e9
EPS = 1e-5


LOCAL_HEADS, LOCAL_WINDOW, LOCAL_DILATION = 32, 8, 2

NPRE = 10
AHEAD = 4
WO_AT = 11
REORDER_AT, FIRST_QKV_AT = 8, 17
LAG = {"first": 2, "second": 3, "ramp": 2, "full": 1, "tail": 2}


def _ln(xf):
    m = jnp.mean(xf, axis=-1, keepdims=True)
    d = xf - m
    v = jnp.mean(d * d, axis=-1, keepdims=True)
    return d * lax.rsqrt(v + EPS)


def _recip(x):
    r = pl.reciprocal(x, approx=True)
    return r * (2.0 - x * r)


def _dot(a, b):
    return jnp.dot(a, b, preferred_element_type=F32)


def _dot_nt(a, b):
    return lax.dot_general(a, b, NT_DIMS, preferred_element_type=F32)


def _unpack(w32):
    return pltpu.bitcast(w32, BF16)


def _pack(x):
    return pltpu.bitcast(x.astype(BF16), I32)


def _prow(start, size):
    return pl.ds(start // 2, size // 2) if isinstance(start, int) else pl.ds(pl.multiple_of(start // 2, 8), size // 2)


def _kernel(x_hbm, mem0_ref, wq_hbm, wk_hbm, wv_hbm, wo_hbm, bw_hbm, bo_hbm, out_hbm,
            r_ref, h_ref, o_ref, bwp_ref, bop_ref, qb_ref, kb_ref, vb_ref, acc_ref,
            sq_ref, sk_ref, sv_ref, wq_ref, wk_ref, wv_ref, wo_ref, bw_ref, bo_ref,
            hpre_ref, pq_ref, pk_ref, pv_ref, tr_ref, sems, psems,
            *, S, D, H, DH, M, SEG):
    BH, BW, BDIL = LOCAL_HEADS, LOCAL_WINDOW, LOCAL_DILATION
    NS = S // SEG
    NP = H // 2
    PW = 2 * DH
    T1, T3, T4 = 2 * M, 2 * M + SEG, 2 * M + 2 * SEG
    NK = T4 + T1
    PAD = 3
    BDH = D // BH
    HALO = 16
    NT = D // 128
    a_scale = DH ** -0.5
    b_scale = BDH ** -0.5
    XH = (NPRE + 1) * SEG

    cp_bw = pltpu.make_async_copy(bw_hbm, bw_ref, sems.at[0])
    cp_bo = pltpu.make_async_copy(bo_hbm, bo_ref, sems.at[1])
    cp_xh = pltpu.make_async_copy(x_hbm.at[0:XH], r_ref.at[PAD * SEG:PAD * SEG + XH], sems.at[2])
    cp_xt = pltpu.make_async_copy(x_hbm.at[XH:S], r_ref.at[PAD * SEG + XH:PAD * SEG + S], sems.at[3])
    cp_wo = pltpu.make_async_copy(wo_hbm, wo_ref, sems.at[4])

    def pair_copies(p):
        rows = pl.ds(pl.multiple_of(p * PW, PW), PW)
        return [pltpu.make_async_copy(w.at[rows], s.at[rows], psems.at[p])
                for w, s in ((wq_hbm, sq_ref), (wk_hbm, sk_ref), (wv_hbm, sv_ref))]

    def seg(i):
        return pl.ds(pl.multiple_of((i + PAD) * SEG, SEG), SEG)

    def out_copy(i):
        return pltpu.make_async_copy(
            r_ref.at[seg(i)], out_hbm.at[pl.ds(pl.multiple_of(i * SEG, SEG), SEG)], sems.at[5])

    cp_xh.start()
    for cp in pair_copies(0):
        cp.start()

    r_ref[0:PAD * SEG, :] = jnp.zeros((PAD * SEG, D), BF16)
    r_ref[(PAD + NS) * SEG:(2 * PAD + NS) * SEG, :] = jnp.zeros((PAD * SEG, D), BF16)
    qb_ref[...] = jnp.zeros(qb_ref.shape, F32)
    kb_ref[...] = jnp.zeros(kb_ref.shape, F32)
    vb_ref[...] = jnp.zeros(vb_ref.shape, F32)
    mem0 = mem0_ref[...].astype(F32)
    mem00 = jnp.concatenate([mem0, mem0], axis=0)
    h_ref[0, _prow(0, T1), :] = _pack(mem00)
    cp_xh.wait()
    for p in range(1, AHEAD):
        for cp in pair_copies(p):
            cp.start()
    hpre_ref[...] = _pack(_ln(r_ref[PAD * SEG:(PAD + NPRE) * SEG, :].astype(F32)))

    def pair_prologue(p, _):
        for cp in pair_copies(p):
            cp.wait()

        @pl.when(p + AHEAD < NP)
        def _():
            for cp in pair_copies(p + AHEAD):
                cp.start()

        @pl.when(p == WO_AT)
        def _():
            cp_wo.start()

        rows = pl.ds(pl.multiple_of(p * PW, PW), PW)
        cols = pl.ds(pl.multiple_of(p * PW, 128), PW)
        hp = _unpack(hpre_ref[_prow(0, (NPRE - 2) * SEG), :])
        for s_ref, w_ref, p_ref in ((sq_ref, wq_ref, pq_ref), (sk_ref, wk_ref, pk_ref),
                                    (sv_ref, wv_ref, pv_ref)):
            w = s_ref[rows, :]
            p_ref[_prow(0, (NPRE - 2) * SEG), cols] = _pack(_dot_nt(hp, w))
            w_ref[:, cols] = pltpu.bitcast(w.T, I32)
        return 0

    lax.fori_loop(0, NP, pair_prologue, 0)

    def gather_rows(base):
        return jnp.concatenate(
            [tr_ref[pl.ds(base + j, BH, stride=BDH), :] for j in range(BDH)], axis=0)

    def reorder_local_weights():
        cp_bw.wait()
        cp_bo.wait()
        tr_ref[3 * D:3 * D + BH, :] = jnp.zeros((BH, 128), F32)
        for kt in range(NT):
            tr_ref[0:3 * D, :] = bw_ref[kt * 128:(kt + 1) * 128, :].T.astype(F32)
            for m in range(3):
                g = gather_rows(m * D).astype(BF16).T
                bwp_ref[kt * 64:(kt + 1) * 64, m * D:(m + 1) * D] = pltpu.bitcast(g, I32)
        for lt in range(NT):
            tr_ref[0:D, :] = bo_ref[:, lt * 128:(lt + 1) * 128].astype(F32)
            bop_ref[:, lt * 128:(lt + 1) * 128] = _pack(gather_rows(0))

    def b_seg(t, l):
        return t - 1 - 2 * l

    def b_local_attn(t, slots, masked=True):
        blocks = []
        for l in slots:
            for rb in range(SEG // 8):
                pos = lax.broadcasted_iota(I32, (8, 128), 0) + (b_seg(t, l) * SEG + rb * 8)
                qs = [qb_ref[l, c, rb * 8:rb * 8 + 8, :] for c in range(NT)]
                logits = []
                for w in range(BW):
                    r0 = HALO - BDIL * w + rb * 8
                    a = None
                    for c in range(NT):
                        pr = qs[c] * kb_ref[l, c, r0:r0 + 8, :]
                        a = pr if a is None else a + pr
                    a = a + pltpu.roll(a, 64, 1)
                    a = a + pltpu.roll(a, 32, 1)
                    logits.append(jnp.where(pos >= BDIL * w, a, NEG) if (masked and BDIL * w > rb * 8) else a)
                mx = logits[0]
                for w in range(1, BW):
                    mx = jnp.maximum(mx, logits[w])
                es = [jnp.exp(a - mx) for a in logits]
                sm = es[0]
                for w in range(1, BW):
                    sm = sm + es[w]
                inv = _recip(sm)
                aws = [e * inv for e in es]
                tiles = []
                for c in range(NT):
                    ob = None
                    for w in range(BW):
                        r0 = HALO - BDIL * w + rb * 8
                        term = aws[w] * vb_ref[l, c, r0:r0 + 8, :]
                        ob = term if ob is None else ob + term
                    tiles.append(ob)
                blocks.append(jnp.concatenate(tiles, axis=1))
        return jnp.concatenate(blocks, axis=0).astype(BF16)

    def b_out(t, slots, ob):
        bout = _dot(ob, _unpack(bop_ref[...]))
        news = []
        for i, l in enumerate(slots):
            sg = seg(b_seg(t, l))
            new = (r_ref[sg, :].astype(F32) + bout[i * SEG:(i + 1) * SEG]).astype(BF16)
            r_ref[sg, :] = new
            news.append(new)
        return news

    def b_qkv(slots, xs):
        hb = jnp.concatenate([_ln(x.astype(F32)) for x in xs], axis=0).astype(BF16)
        qkv = _dot(hb, _unpack(bwp_ref[...]))
        for i, l in enumerate(slots):
            rows = slice(i * SEG, (i + 1) * SEG)
            for c in range(NT):
                c0 = c * 128
                qb_ref[l, c] = qkv[rows, c0:c0 + 128] * b_scale
                kb_ref[l, c, 0:HALO, :] = kb_ref[l, c, SEG:SEG + HALO, :]
                vb_ref[l, c, 0:HALO, :] = vb_ref[l, c, SEG:SEG + HALO, :]
                kb_ref[l, c, HALO:HALO + SEG, :] = qkv[rows, D + c0:D + c0 + 128]
                vb_ref[l, c, HALO:HALO + SEG, :] = qkv[rows, 2 * D + c0:2 * D + c0 + 128]

    def softmax(s, mask):
        s = jnp.where(mask, s * a_scale, NEG)
        mx = jnp.max(s, axis=-1, keepdims=True)
        e = jnp.exp(s - mx)
        return e * _recip(jnp.sum(e, axis=-1, keepdims=True))

    def split_lo_hi(z):
        rows = z.shape[0]
        lo32 = jnp.where(lax.broadcasted_iota(I32, (rows // 2, 128), 1) < 64, I32(-1), I32(0))
        zi = pltpu.bitcast(z, I32)
        return pltpu.bitcast(zi & lo32, BF16), pltpu.bitcast(zi & ~lo32, BF16)

    def step(t, kind):
        lag = LAG[kind]
        head = kind in ("first", "second")
        slot = t % 2 if head else lax.rem(t, 2)
        nslot = 1 - slot
        both = kind in ("ramp", "full")
        lay = 0 if head else 1
        RW = T4 if both else T3
        if kind == "full":
            hrows = _unpack(h_ref[slot])
        elif head:
            arows = _prow((NPRE - 2 + t) * SEG, SEG)
            hrows = _unpack(jnp.concatenate([h_ref[slot, _prow(0, T1), :], hpre_ref[arows, :]], axis=0))
        else:
            hrows = _unpack(jnp.concatenate([h_ref[slot, _prow(0, T1), :], h_ref[slot, _prow(T3, SEG), :]], axis=0))
        b_attn_slots = (0,) if head else (0, 1)
        b_qkv_slots = (0,) if head else (1,) if kind == "tail" else (0, 1)

        ri = lax.broadcasted_iota(I32, (RW, NK), 0)
        ci = lax.broadcasted_iota(I32, (RW, NK), 1)
        if both:
            def layer(i):
                return jnp.where(i < M, 0, jnp.where(i < T1, 1, jnp.where(i < T3, 0, 1)))

            def allowed(kidx, kvalid):
                return kvalid & (layer(ri) == layer(kidx)) & ((ri < T1) | (kidx < T1) | (ri >= kidx))
            mask0 = allowed(ci, ci < T4)
            nat1 = jnp.where(ci < T3, ci - T1 + T3, jnp.where(ci < T4, ci - T3 + T1, ci - T4))
            mask1 = allowed(nat1, ci >= T1)

            def shared_w(z):
                zl, zh = split_lo_hi(z)
                w1 = jnp.concatenate([zl[0:T3], zh[T1:T3], zh[0:T1]], axis=0)
                w3 = jnp.concatenate([zl[0:T1], zh[T3:T4], zl[T3:T4], zh[0:T1]], axis=0)
                return w1, w3

            def h0_rows(z):
                return jnp.concatenate([z, z[0:T1]], axis=0)

            def h1_rows(z):
                return jnp.concatenate([z[0:T1], z[T3:T4], z[T1:T3], z[0:T1]], axis=0)

            def shared(dot, lhs, ws):
                y1 = dot(lhs[0:T3], ws[0])
                y3 = dot(jnp.concatenate([lhs[0:T1], lhs[T3:T4]], axis=0), ws[1])
                return jnp.concatenate([y1[0:M], y3[M:T1], y1[T1:T3], y3[T1:T3]], axis=0)
        else:
            def allowed(kidx, kvalid):
                kok = kvalid & ((kidx >= T1) | (kidx // M == lay))
                return kok & ((ri < T1) | (kidx < T1) | (ri >= kidx))
            mask0 = allowed(ci, ci < T3)
            nat1 = jnp.where(ci < T4, ci - T3 + T1, ci - T4)
            mask1 = allowed(nat1, ci >= T3)

            def shared_w(z):
                zl, zh = split_lo_hi(z)
                return (jnp.concatenate([zl, zh[T1:T3], zh[0:T1]], axis=0),)

            def h0_rows(z):
                return jnp.concatenate([z, z], axis=0)

            def h1_rows(z):
                return jnp.concatenate([z, z[T1:T3], z[0:T1]], axis=0)

            def shared(dot, lhs, ws):
                return dot(lhs, ws[0])

        def proj(w_ref, pre_ref, p):
            c0 = p * PW
            y = _dot(hrows, _unpack(w_ref[:, c0:c0 + PW])).astype(BF16)
            if kind in ("full", "tail"):
                return y
            pre = _unpack(pre_ref[_prow(t * SEG, SEG), c0:c0 + PW])
            if kind == "ramp":
                return jnp.concatenate([y[0:T1], pre, y[T1:T3]], axis=0)
            pre_ref[arows, c0:c0 + PW] = pltpu.bitcast(y[T1:T3], I32)
            return jnp.concatenate([y[0:T1], pre], axis=0)

        def qk(q, k):
            qA, qB, qC = q[:, 0:128], q[:, 128:256], q[:, 256:384]
            sa = _dot_nt(qA, h0_rows(k[:, 0:128]))
            sc = _dot_nt(qC, h1_rows(k[:, 256:384]))
            x = shared(_dot_nt, qB, shared_w(k[:, 128:256]))
            return sa + x, sc + x

        def pv(p, s0, s1, v):
            c0 = p * PW
            p0 = softmax(s0, mask0)
            p1 = softmax(s1, mask1)
            pm = (p0 + p1).astype(BF16)
            oa = _dot(p0.astype(BF16), h0_rows(v[:, 0:128]))
            oc = _dot(p1.astype(BF16), h1_rows(v[:, 256:384]))
            ob_ = shared(_dot, pm, shared_w(v[:, 128:256]))
            o_ref[_prow(0, RW), c0:c0 + 128] = _pack(oa)
            o_ref[_prow(0, RW), c0 + 128:c0 + 256] = _pack(ob_)
            o_ref[_prow(0, RW), c0 + 256:c0 + 384] = _pack(oc)

        def out_chunk(c0, c1):
            return _dot(_unpack(o_ref[_prow(0, RW), c0 * PW:c1 * PW]), wo_ref[c0 * PW:c1 * PW, :])

        if not head:
            ob = b_local_attn(t, b_attn_slots, masked=kind == "ramp")

        qs, ks, vs, ss = {}, {}, {}, {}
        cuts = [0, (NP + 1 - lag) // 2] + [NP - lag + s for s in range(1, lag)]
        for p in range(NP + lag):
            if 1 <= p <= NP:
                ss[p - 1] = qk(qs.pop(p - 1), ks.pop(p - 1))
            if p < NP:
                qs[p] = proj(wq_ref, pq_ref, p)
                ks[p] = proj(wk_ref, pk_ref, p)
            elif p == NP:
                if kind == "first":
                    cp_wo.wait()
                    cp_bw.start()
                    cp_bo.start()
                    cp_xt.start()
                acc_ref[0:RW] = out_chunk(cuts[0], cuts[1])
            else:
                acc_ref[0:RW] += out_chunk(cuts[p - NP], cuts[p - NP + 1])
            if p >= lag:
                pv(p - lag, *ss.pop(p - lag), vs.pop(p - lag))
            if p < NP:
                vs[p] = proj(wv_ref, pv_ref, p)
            if kind == "second" and p == REORDER_AT:
                reorder_local_weights()
            if kind == "second" and p == FIRST_QKV_AT:
                b_qkv((0,), [r_ref[seg(0), :]])
                ob = b_local_attn(t, b_attn_slots, masked=True)
        aout = acc_ref[0:RW] + out_chunk(cuts[lag], NP)

        def add_residual(i, rows):
            new = (r_ref[seg(i), :].astype(F32) + aout[rows]).astype(BF16)
            r_ref[seg(i), :] = new
            return new

        if head:
            xs = [add_residual(t, slice(T1, T3))]
        elif kind == "tail":
            xs = [add_residual(t - 2, slice(T1, T3))]
        else:
            xs = [add_residual(t, slice(T1, T3)), add_residual(t - 2, slice(T3, T4))]
        mrow = lax.broadcasted_iota(I32, (T1, D), 0)
        mem_next = jnp.where(mrow < M, aout[0:T1], mem00) if head else aout[0:T1]
        h_ref[nslot, _prow(0, T1), :] = _pack(mem_next)
        if both:
            h_ref[nslot, _prow(T1, SEG), :] = _pack(_ln(r_ref[seg(t + 1), :].astype(F32)))
        if kind == "first":
            return

        news = b_out(t, b_attn_slots, ob)
        h_ref[nslot, _prow(T3, SEG), :] = _pack(_ln(news[0].astype(F32)))
        b_qkv(b_qkv_slots, xs)
        if not head:
            @pl.when(t >= 3)
            def _():
                out_copy(t - 3).start()

    def loop(lo, hi, kind):
        def body(t, _):
            step(t, kind)
            return 0
        lax.fori_loop(lo, hi, body, 0)

    step(0, "first")
    step(1, "second")
    loop(2, NPRE, "ramp")
    cp_xt.wait()
    loop(NPRE, NS, "full")
    loop(NS, NS + 2, "tail")
    b_out(NS + 2, (1,), b_local_attn(NS + 2, (1,), masked=False))
    out_copy(NS - 1).start()
    pltpu.make_async_copy(r_ref.at[PAD * SEG:(PAD + NS) * SEG], out_hbm, sems.at[5]).wait()


@functools.partial(jax.jit, static_argnames=("A_seg_len",))
def pallas_interleave_layers__memory_aug_recurrent_mem_tr__sliding_local_dilated__prompt_kernel(A_x, A_mem0, A_Wq, A_Wk, A_Wv, A_Wo, A_seg_len, B_x, B_wqkv, B_wo):
    del B_x
    B, S, D = A_x.shape
    M = A_mem0.shape[1]
    _, H, DH = A_Wq.shape
    SEG = A_seg_len
    HD = H * DH
    x = A_x.reshape(S, D)
    mem0 = A_mem0.reshape(M, D)
    wq = jnp.transpose(A_Wq, (1, 2, 0)).reshape(HD, D)
    wk = jnp.transpose(A_Wk, (1, 2, 0)).reshape(HD, D)
    wv = jnp.transpose(A_Wv, (1, 2, 0)).reshape(HD, D)
    wo = A_Wo.reshape(HD, D)
    R2 = 2 * M + 2 * SEG
    kern = functools.partial(_kernel, S=S, D=D, H=H, DH=DH, M=M, SEG=SEG)
    hbm = pl.BlockSpec(memory_space=pl.ANY)
    out = pl.pallas_call(
        kern,
        out_shape=jax.ShapeDtypeStruct((S, D), BF16),
        in_specs=[hbm, pl.BlockSpec(memory_space=pltpu.VMEM)] + [hbm] * 6,
        out_specs=hbm,
        scratch_shapes=[
            pltpu.VMEM((S + 6 * SEG, D), BF16),
            pltpu.VMEM((2, R2 // 2, D), I32),
            pltpu.VMEM((R2 // 2, HD), I32),
            pltpu.VMEM((D // 2, 3 * D), I32),
            pltpu.VMEM((D // 2, D), I32),
            pltpu.VMEM((2, D // 128, SEG, 128), F32),
            pltpu.VMEM((2, D // 128, 16 + SEG, 128), F32),
            pltpu.VMEM((2, D // 128, 16 + SEG, 128), F32),
            pltpu.VMEM((R2, D), F32),
            pltpu.VMEM((HD, D), BF16),
            pltpu.VMEM((HD, D), BF16),
            pltpu.VMEM((HD, D), BF16),
            pltpu.VMEM((D // 2, HD), I32),
            pltpu.VMEM((D // 2, HD), I32),
            pltpu.VMEM((D // 2, HD), I32),
            pltpu.VMEM((HD, D), BF16),
            pltpu.VMEM((D, 3 * D), BF16),
            pltpu.VMEM((D, D), BF16),
            pltpu.VMEM((NPRE * SEG // 2, D), I32),
            pltpu.VMEM((NPRE * SEG // 2, HD), I32),
            pltpu.VMEM((NPRE * SEG // 2, HD), I32),
            pltpu.VMEM((NPRE * SEG // 2, HD), I32),
            pltpu.VMEM((3 * D + LOCAL_HEADS, 128), F32),
            pltpu.SemaphoreType.DMA((6,)),
            pltpu.SemaphoreType.DMA((H // 2,)),
        ],
        compiler_params=pltpu.CompilerParams(
            vmem_limit_bytes=120 * 2**20,
            flags={"XLA_TPU_EVENLY_DISTRIBUTE_CRITICAL_NODES": True}),
    )(x, mem0, wq, wk, wv, wo, B_wqkv, B_wo)
    return out.reshape(B, S, D)
```

```python
import functools

import jax
import jax.numpy as jnp
from jax import lax
from jax.experimental import pallas as pl
from jax.experimental.pallas import tpu as pltpu

F32 = jnp.float32
BF16 = jnp.bfloat16
I32 = jnp.int32
NT_DIMS = (((1,), (1,)), ((), ()))
NEG = -1e9
EPS = 1e-5


LOCAL_HEADS, LOCAL_WINDOW, LOCAL_DILATION = 32, 8, 2

NPRE = 10
AHEAD = 4
WO_AT = 11
REORDER_AT, FIRST_QKV_AT = 8, 17
LAG = {"first": 2, "second": 3, "ramp": 2, "full": 1, "tail": 2, "last": 2}


def _ln(xf):
    m = jnp.mean(xf, axis=-1, keepdims=True)
    d = xf - m
    v = jnp.mean(d * d, axis=-1, keepdims=True)
    return d * lax.rsqrt(v + EPS)


def _recip(x):
    r = pl.reciprocal(x, approx=True)
    return r * (2.0 - x * r)


def _dot(a, b):
    return jnp.dot(a, b, preferred_element_type=F32)


def _dot_nt(a, b):
    return lax.dot_general(a, b, NT_DIMS, preferred_element_type=F32)


def _unpack(w32):
    return pltpu.bitcast(w32, BF16)


def _pack(x):
    return pltpu.bitcast(x.astype(BF16), I32)


def _prow(start, size):
    return pl.ds(start // 2, size // 2) if isinstance(start, int) else pl.ds(pl.multiple_of(start // 2, 8), size // 2)


def _kernel(x_hbm, mem0_ref, wq_hbm, wk_hbm, wv_hbm, wo_hbm, bw_hbm, bo_hbm, out_hbm,
            r_ref, h_ref, o_ref, bwp_ref, bop_ref, qb_ref, kb_ref, vb_ref, acc_ref,
            sq_ref, sk_ref, sv_ref, wq_ref, wk_ref, wv_ref, wo_ref, bw_ref, bo_ref,
            hpre_ref, pq_ref, pk_ref, pv_ref, tr_ref, sems, psems,
            *, S, D, H, DH, M, SEG):
    BH, BW, BDIL = LOCAL_HEADS, LOCAL_WINDOW, LOCAL_DILATION
    NS = S // SEG
    NP = H // 2
    PW = 2 * DH
    T1, T3, T4 = 2 * M, 2 * M + SEG, 2 * M + 2 * SEG
    NK = T4 + T1
    PAD = 3
    BDH = D // BH
    HALO = 16
    NT = D // 128
    a_scale = DH ** -0.5
    b_scale = BDH ** -0.5
    XH = (NPRE + 1) * SEG

    cp_bw = pltpu.make_async_copy(bw_hbm, bw_ref, sems.at[0])
    cp_bo = pltpu.make_async_copy(bo_hbm, bo_ref, sems.at[1])
    cp_xh = pltpu.make_async_copy(x_hbm.at[0:XH], r_ref.at[PAD * SEG:PAD * SEG + XH], sems.at[2])
    cp_xt = pltpu.make_async_copy(x_hbm.at[XH:S], r_ref.at[PAD * SEG + XH:PAD * SEG + S], sems.at[3])
    cp_wo = pltpu.make_async_copy(wo_hbm, wo_ref, sems.at[4])

    def pair_copies(p):
        rows = pl.ds(pl.multiple_of(p * PW, PW), PW)
        return [pltpu.make_async_copy(w.at[rows], s.at[rows], psems.at[p])
                for w, s in ((wq_hbm, sq_ref), (wk_hbm, sk_ref), (wv_hbm, sv_ref))]

    def seg(i):
        return pl.ds(pl.multiple_of((i + PAD) * SEG, SEG), SEG)

    def out_copy(i):
        return pltpu.make_async_copy(
            r_ref.at[seg(i)], out_hbm.at[pl.ds(pl.multiple_of(i * SEG, SEG), SEG)], sems.at[5])

    cp_xh.start()
    for cp in pair_copies(0):
        cp.start()

    r_ref[0:PAD * SEG, :] = jnp.zeros((PAD * SEG, D), BF16)
    r_ref[(PAD + NS) * SEG:(2 * PAD + NS) * SEG, :] = jnp.zeros((PAD * SEG, D), BF16)
    qb_ref[...] = jnp.zeros(qb_ref.shape, F32)
    kb_ref[...] = jnp.zeros(kb_ref.shape, F32)
    vb_ref[...] = jnp.zeros(vb_ref.shape, F32)
    mem0 = mem0_ref[...].astype(F32)
    mem00 = jnp.concatenate([mem0, mem0], axis=0)
    h_ref[0, _prow(0, T1), :] = _pack(mem00)
    cp_xh.wait()
    for p in range(1, AHEAD):
        for cp in pair_copies(p):
            cp.start()
    hpre_ref[...] = _pack(_ln(r_ref[PAD * SEG:(PAD + NPRE) * SEG, :].astype(F32)))

    def pair_prologue(p, _):
        for cp in pair_copies(p):
            cp.wait()

        @pl.when(p + AHEAD < NP)
        def _():
            for cp in pair_copies(p + AHEAD):
                cp.start()

        @pl.when(p == WO_AT)
        def _():
            cp_wo.start()

        rows = pl.ds(pl.multiple_of(p * PW, PW), PW)
        cols = pl.ds(pl.multiple_of(p * PW, 128), PW)
        hp = _unpack(hpre_ref[_prow(0, (NPRE - 2) * SEG), :])
        for s_ref, w_ref, p_ref in ((sq_ref, wq_ref, pq_ref), (sk_ref, wk_ref, pk_ref),
                                    (sv_ref, wv_ref, pv_ref)):
            w = s_ref[rows, :]
            p_ref[_prow(0, (NPRE - 2) * SEG), cols] = _pack(_dot_nt(hp, w))
            w_ref[:, cols] = pltpu.bitcast(w.T, I32)
        return 0

    lax.fori_loop(0, NP, pair_prologue, 0)

    def gather_rows(base):
        return jnp.concatenate(
            [tr_ref[pl.ds(base + j, BH, stride=BDH), :] for j in range(BDH)], axis=0)

    def reorder_local_weights():
        cp_bw.wait()
        cp_bo.wait()
        tr_ref[3 * D:3 * D + BH, :] = jnp.zeros((BH, 128), F32)
        for kt in range(NT):
            tr_ref[0:3 * D, :] = bw_ref[kt * 128:(kt + 1) * 128, :].T.astype(F32)
            for m in range(3):
                g = gather_rows(m * D).astype(BF16).T
                bwp_ref[kt * 64:(kt + 1) * 64, m * D:(m + 1) * D] = pltpu.bitcast(g, I32)
        for lt in range(NT):
            tr_ref[0:D, :] = bo_ref[:, lt * 128:(lt + 1) * 128].astype(F32)
            bop_ref[:, lt * 128:(lt + 1) * 128] = _pack(gather_rows(0))

    def b_seg(t, l):
        return t - 1 - 2 * l

    def b_local_attn(t, slots, masked=True):
        blocks = []
        for l in slots:
            for rb in range(SEG // 8):
                pos = lax.broadcasted_iota(I32, (8, 128), 0) + (b_seg(t, l) * SEG + rb * 8)
                qs = [qb_ref[l, c, rb * 8:rb * 8 + 8, :] for c in range(NT)]
                logits = []
                for w in range(BW):
                    r0 = HALO - BDIL * w + rb * 8
                    a = None
                    for c in range(NT):
                        pr = qs[c] * kb_ref[l, c, r0:r0 + 8, :]
                        a = pr if a is None else a + pr
                    a = a + pltpu.roll(a, 64, 1)
                    a = a + pltpu.roll(a, 32, 1)
                    logits.append(jnp.where(pos >= BDIL * w, a, NEG) if (masked and BDIL * w > rb * 8) else a)
                mx = logits[0]
                for w in range(1, BW):
                    mx = jnp.maximum(mx, logits[w])
                es = [jnp.exp(a - mx) for a in logits]
                sm = es[0]
                for w in range(1, BW):
                    sm = sm + es[w]
                inv = _recip(sm)
                aws = [e * inv for e in es]
                tiles = []
                for c in range(NT):
                    ob = None
                    for w in range(BW):
                        r0 = HALO - BDIL * w + rb * 8
                        term = aws[w] * vb_ref[l, c, r0:r0 + 8, :]
                        ob = term if ob is None else ob + term
                    tiles.append(ob)
                blocks.append(jnp.concatenate(tiles, axis=1))
        return jnp.concatenate(blocks, axis=0).astype(BF16)

    def b_out(t, slots, ob):
        bout = _dot(ob, _unpack(bop_ref[...]))
        news = []
        for i, l in enumerate(slots):
            sg = seg(b_seg(t, l))
            new = (r_ref[sg, :].astype(F32) + bout[i * SEG:(i + 1) * SEG]).astype(BF16)
            r_ref[sg, :] = new
            news.append(new)
        return news

    def b_qkv(slots, xs):
        hb = jnp.concatenate([_ln(x.astype(F32)) for x in xs], axis=0).astype(BF16)
        qkv = _dot(hb, _unpack(bwp_ref[...]))
        for i, l in enumerate(slots):
            rows = slice(i * SEG, (i + 1) * SEG)
            for c in range(NT):
                c0 = c * 128
                qb_ref[l, c] = qkv[rows, c0:c0 + 128] * b_scale
                kb_ref[l, c, 0:HALO, :] = kb_ref[l, c, SEG:SEG + HALO, :]
                vb_ref[l, c, 0:HALO, :] = vb_ref[l, c, SEG:SEG + HALO, :]
                kb_ref[l, c, HALO:HALO + SEG, :] = qkv[rows, D + c0:D + c0 + 128]
                vb_ref[l, c, HALO:HALO + SEG, :] = qkv[rows, 2 * D + c0:2 * D + c0 + 128]

    def softmax(s, mask):
        s = jnp.where(mask, s * a_scale, NEG)
        mx = jnp.max(s, axis=-1, keepdims=True)
        e = jnp.exp(s - mx)
        return e * _recip(jnp.sum(e, axis=-1, keepdims=True))

    def split_lo_hi(z):
        rows = z.shape[0]
        lo32 = jnp.where(lax.broadcasted_iota(I32, (rows // 2, 128), 1) < 64, I32(-1), I32(0))
        zi = pltpu.bitcast(z, I32)
        return pltpu.bitcast(zi & lo32, BF16), pltpu.bitcast(zi & ~lo32, BF16)

    def step(t, kind):
        lag = LAG[kind]
        head = kind in ("first", "second")
        slot = t % 2 if isinstance(t, int) else lax.rem(t, 2)
        nslot = 1 - slot
        both = kind in ("ramp", "full")
        lay = 0 if head else 1
        last = kind == "last"
        RK = T4 if both else T3
        R0 = T1 if last else 0
        RW = RK - R0
        if kind == "full":
            hrows = _unpack(h_ref[slot])
        elif head:
            arows = _prow((NPRE - 2 + t) * SEG, SEG)
            hrows = _unpack(jnp.concatenate([h_ref[slot, _prow(0, T1), :], hpre_ref[arows, :]], axis=0))
        else:
            hrows = _unpack(jnp.concatenate([h_ref[slot, _prow(0, T1), :], h_ref[slot, _prow(T3, SEG), :]], axis=0))
        b_attn_slots = (0,) if head else (1,) if last else (0, 1)
        b_qkv_slots = (0,) if head else (0, 1) if both else (1,)

        ri = lax.broadcasted_iota(I32, (RW, NK), 0) + R0
        ci = lax.broadcasted_iota(I32, (RW, NK), 1)
        if both:
            def layer(i):
                return jnp.where(i < M, 0, jnp.where(i < T1, 1, jnp.where(i < T3, 0, 1)))

            def allowed(kidx, kvalid):
                return kvalid & (layer(ri) == layer(kidx)) & ((ri < T1) | (kidx < T1) | (ri >= kidx))
            mask0 = allowed(ci, ci < T4)
            nat1 = jnp.where(ci < T3, ci - T1 + T3, jnp.where(ci < T4, ci - T3 + T1, ci - T4))
            mask1 = allowed(nat1, ci >= T1)

            def shared_w(z):
                zl, zh = split_lo_hi(z)
                w1 = jnp.concatenate([zl[0:T3], zh[T1:T3], zh[0:T1]], axis=0)
                w3 = jnp.concatenate([zl[0:T1], zh[T3:T4], zl[T3:T4], zh[0:T1]], axis=0)
                return w1, w3

            def h0_rows(z):
                return jnp.concatenate([z, z[0:T1]], axis=0)

            def h1_rows(z):
                return jnp.concatenate([z[0:T1], z[T3:T4], z[T1:T3], z[0:T1]], axis=0)

            def shared(dot, lhs, ws):
                y1 = dot(lhs[0:T3], ws[0])
                y3 = dot(jnp.concatenate([lhs[0:T1], lhs[T3:T4]], axis=0), ws[1])
                return jnp.concatenate([y1[0:M], y3[M:T1], y1[T1:T3], y3[T1:T3]], axis=0)
        else:
            def allowed(kidx, kvalid):
                kok = kvalid & ((kidx >= T1) | (kidx // M == lay))
                return kok & ((ri < T1) | (kidx < T1) | (ri >= kidx))
            mask0 = allowed(ci, ci < T3)
            nat1 = jnp.where(ci < T4, ci - T3 + T1, ci - T4)
            mask1 = allowed(nat1, ci >= T3)

            def shared_w(z):
                zl, zh = split_lo_hi(z)
                return (jnp.concatenate([zl, zh[T1:T3], zh[0:T1]], axis=0),)

            def h0_rows(z):
                return jnp.concatenate([z, z], axis=0)

            def h1_rows(z):
                return jnp.concatenate([z, z[T1:T3], z[0:T1]], axis=0)

            def shared(dot, lhs, ws):
                return dot(lhs, ws[0])

        def proj(w_ref, pre_ref, p):
            c0 = p * PW
            y = _dot(hrows, _unpack(w_ref[:, c0:c0 + PW])).astype(BF16)
            if kind in ("full", "tail", "last"):
                return y
            pre = _unpack(pre_ref[_prow(t * SEG, SEG), c0:c0 + PW])
            if kind == "ramp":
                return jnp.concatenate([y[0:T1], pre, y[T1:T3]], axis=0)
            pre_ref[arows, c0:c0 + PW] = pltpu.bitcast(y[T1:T3], I32)
            return jnp.concatenate([y[0:T1], pre], axis=0)

        def qk(q, k):
            qA, qB, qC = q[:, 0:128], q[:, 128:256], q[:, 256:384]
            sa = _dot_nt(qA, h0_rows(k[:, 0:128]))
            sc = _dot_nt(qC, h1_rows(k[:, 256:384]))
            x = shared(_dot_nt, qB, shared_w(k[:, 128:256]))
            return sa + x, sc + x

        def pv(p, s0, s1, v):
            c0 = p * PW
            p0 = softmax(s0, mask0)
            p1 = softmax(s1, mask1)
            pm = (p0 + p1).astype(BF16)
            oa = _dot(p0.astype(BF16), h0_rows(v[:, 0:128]))
            oc = _dot(p1.astype(BF16), h1_rows(v[:, 256:384]))
            ob_ = shared(_dot, pm, shared_w(v[:, 128:256]))
            o_ref[_prow(0, RW), c0:c0 + 128] = _pack(oa)
            o_ref[_prow(0, RW), c0 + 128:c0 + 256] = _pack(ob_)
            o_ref[_prow(0, RW), c0 + 256:c0 + 384] = _pack(oc)

        def out_chunk(c0, c1):
            return _dot(_unpack(o_ref[_prow(0, RW), c0 * PW:c1 * PW]), wo_ref[c0 * PW:c1 * PW, :])

        if not head:
            ob = b_local_attn(t, b_attn_slots, masked=kind == "ramp")

        qs, ks, vs, ss = {}, {}, {}, {}
        cuts = [0, (NP + 1 - lag) // 2] + [NP - lag + s for s in range(1, lag)]
        for p in range(NP + lag):
            if 1 <= p <= NP:
                ss[p - 1] = qk(qs.pop(p - 1), ks.pop(p - 1))
            if p < NP:
                if last:
                    qs[p] = _dot(hrows[T1:T3], _unpack(wq_ref[:, p * PW:(p + 1) * PW])).astype(BF16)
                else:
                    qs[p] = proj(wq_ref, pq_ref, p)
                ks[p] = proj(wk_ref, pk_ref, p)
            elif p == NP:
                if kind == "first":
                    cp_wo.wait()
                    cp_bw.start()
                    cp_bo.start()
                    cp_xt.start()
                acc_ref[0:RW] = out_chunk(cuts[0], cuts[1])
            else:
                acc_ref[0:RW] += out_chunk(cuts[p - NP], cuts[p - NP + 1])
            if p >= lag:
                pv(p - lag, *ss.pop(p - lag), vs.pop(p - lag))
            if p < NP:
                vs[p] = proj(wv_ref, pv_ref, p)
            if kind == "second" and p == REORDER_AT:
                reorder_local_weights()
            if kind == "second" and p == FIRST_QKV_AT:
                b_qkv((0,), [r_ref[seg(0), :]])
                ob = b_local_attn(t, b_attn_slots, masked=True)
        aout = acc_ref[0:RW] + out_chunk(cuts[lag], NP)

        def add_residual(i, rows):
            new = (r_ref[seg(i), :].astype(F32) + aout[rows]).astype(BF16)
            r_ref[seg(i), :] = new
            return new

        if head:
            xs = [add_residual(t, slice(T1, T3))]
        elif last:
            b_qkv_final = [add_residual(t - 2, slice(0, SEG))]
            b_out(t, b_attn_slots, ob)
            b_qkv(b_qkv_slots, b_qkv_final)
            out_copy(t - 3).start()
            return
        elif kind == "tail":
            xs = [add_residual(t - 2, slice(T1, T3))]
        else:
            xs = [add_residual(t, slice(T1, T3)), add_residual(t - 2, slice(T3, T4))]
        mrow = lax.broadcasted_iota(I32, (T1, D), 0)
        mem_next = jnp.where(mrow < M, aout[0:T1], mem00) if head else aout[0:T1]
        h_ref[nslot, _prow(0, T1), :] = _pack(mem_next)
        if both:
            h_ref[nslot, _prow(T1, SEG), :] = _pack(_ln(r_ref[seg(t + 1), :].astype(F32)))
        if kind == "first":
            return

        news = b_out(t, b_attn_slots, ob)
        h_ref[nslot, _prow(T3, SEG), :] = _pack(_ln(news[0].astype(F32)))
        b_qkv(b_qkv_slots, xs)
        if not head:
            @pl.when(t >= 3)
            def _():
                out_copy(t - 3).start()

    def loop(lo, hi, kind):
        def body(t, _):
            step(t, kind)
            return 0
        lax.fori_loop(lo, hi, body, 0)

    step(0, "first")
    step(1, "second")
    loop(2, NPRE, "ramp")
    cp_xt.wait()
    loop(NPRE, NS, "full")
    step(NS, "tail")
    step(NS + 1, "last")
    b_out(NS + 2, (1,), b_local_attn(NS + 2, (1,), masked=False))
    out_copy(NS - 1).start()
    pltpu.make_async_copy(r_ref.at[PAD * SEG:(PAD + NS) * SEG], out_hbm, sems.at[5]).wait()


@functools.partial(jax.jit, static_argnames=("A_seg_len",))
def pallas_interleave_layers__memory_aug_recurrent_mem_tr__sliding_local_dilated__prompt_kernel(A_x, A_mem0, A_Wq, A_Wk, A_Wv, A_Wo, A_seg_len, B_x, B_wqkv, B_wo):
    del B_x
    B, S, D = A_x.shape
    M = A_mem0.shape[1]
    _, H, DH = A_Wq.shape
    SEG = A_seg_len
    HD = H * DH
    x = A_x.reshape(S, D)
    mem0 = A_mem0.reshape(M, D)
    wq = jnp.transpose(A_Wq, (1, 2, 0)).reshape(HD, D)
    wk = jnp.transpose(A_Wk, (1, 2, 0)).reshape(HD, D)
    wv = jnp.transpose(A_Wv, (1, 2, 0)).reshape(HD, D)
    wo = A_Wo.reshape(HD, D)
    R2 = 2 * M + 2 * SEG
    kern = functools.partial(_kernel, S=S, D=D, H=H, DH=DH, M=M, SEG=SEG)
    hbm = pl.BlockSpec(memory_space=pl.ANY)
    out = pl.pallas_call(
        kern,
        out_shape=jax.ShapeDtypeStruct((S, D), BF16),
        in_specs=[hbm, pl.BlockSpec(memory_space=pltpu.VMEM)] + [hbm] * 6,
        out_specs=hbm,
        scratch_shapes=[
            pltpu.VMEM((S + 6 * SEG, D), BF16),
            pltpu.VMEM((2, R2 // 2, D), I32),
            pltpu.VMEM((R2 // 2, HD), I32),
            pltpu.VMEM((D // 2, 3 * D), I32),
            pltpu.VMEM((D // 2, D), I32),
            pltpu.VMEM((2, D // 128, SEG, 128), F32),
            pltpu.VMEM((2, D // 128, 16 + SEG, 128), F32),
            pltpu.VMEM((2, D // 128, 16 + SEG, 128), F32),
            pltpu.VMEM((R2, D), F32),
            pltpu.VMEM((HD, D), BF16),
            pltpu.VMEM((HD, D), BF16),
            pltpu.VMEM((HD, D), BF16),
            pltpu.VMEM((D // 2, HD), I32),
            pltpu.VMEM((D // 2, HD), I32),
            pltpu.VMEM((D // 2, HD), I32),
            pltpu.VMEM((HD, D), BF16),
            pltpu.VMEM((D, 3 * D), BF16),
            pltpu.VMEM((D, D), BF16),
            pltpu.VMEM((NPRE * SEG // 2, D), I32),
            pltpu.VMEM((NPRE * SEG // 2, HD), I32),
            pltpu.VMEM((NPRE * SEG // 2, HD), I32),
            pltpu.VMEM((NPRE * SEG // 2, HD), I32),
            pltpu.VMEM((3 * D + LOCAL_HEADS, 128), F32),
            pltpu.SemaphoreType.DMA((6,)),
            pltpu.SemaphoreType.DMA((H // 2,)),
        ],
        compiler_params=pltpu.CompilerParams(
            vmem_limit_bytes=120 * 2**20,
            flags={"XLA_TPU_EVENLY_DISTRIBUTE_CRITICAL_NODES": True}),
    )(x, mem0, wq, wk, wv, wo, B_wqkv, B_wo)
    return out.reshape(B, S, D)
```
